```python
import jax
import jax.numpy as jnp

def _softmax(x, axis=-1):
    return jax.nn.softmax(x, axis=axis)

def _gelu(x):
    return jax.nn.gelu(x, approximate=True)

def _silu(x):
    return jax.nn.silu(x)

def _sigmoid(x):
    return jax.nn.sigmoid(x)

def _layernorm(x, axis=-1, eps=1e-05):
    m = jnp.mean(x, axis=axis, keepdims=True)
    v = jnp.var(x, axis=axis, keepdims=True)
    return (x - m) / jnp.sqrt(v + eps)

def _scatter_add(tgt, idx, src, axis=0):
    return tgt.at[idx].add(src)

def _segment_sum(src, seg, n):
    return jax.ops.segment_sum(src, seg, n)

class _Rng:

    def __init__(self, key):
        self._k = key

    def _next(self):
        self._k, sub = jax.random.split(self._k)
        return sub

    def normal(self, shape):
        return jax.random.normal(self._next(), shape, dtype=jnp.bfloat16)

    def randint(self, lo, hi, shape):
        return jax.random.randint(self._next(), shape, lo, hi, dtype=jnp.int32)

    def uniform(self, shape, lo=0.0, hi=1.0):
        return jax.random.uniform(self._next(), shape, jnp.bfloat16, lo, hi)

    def permutation(self, n):
        return jax.random.permutation(self._next(), n)
kernel_name = 'concat_heads__sliding_local_dilated__memory_aug_recurrent_mem_tr__prompt'

def setup_inputs():
    _rng = _Rng(jax.random.key(int.from_bytes(__import__("os").urandom(4), "little")))
    _w = lambda a: (lambda t: t.astype(jnp.bfloat16) if jnp.issubdtype(t.dtype, jnp.floating) else t)(jnp.asarray(a))

    def _A_setup():
        B, S, D = (1, 2048, 640)
        return {'x': _w((lambda *s: _rng.normal(s) * 0.05)(B, S, D)), 'wqkv': _w((lambda *s: _rng.normal(s) * 0.05)(D, 3 * D)), 'wo': _w((lambda *s: _rng.normal(s) * 0.05)(D, D))}
    _A_in = _A_setup()

    def _B_setup():
        B, S, Dm = (1, 2048, 640)
        H, Dh = (32, 192)
        M, seg = (8, 32)
        seg = min(seg, S)
        S = S // seg * seg
        return {'x': _w((lambda *s: _rng.normal(s) * 0.05)(B, S, Dm)), 'mem0': _w((lambda *s: _rng.normal(s) * 0.05)(B, M, Dm)), 'Wq': _w((lambda *s: _rng.normal(s) * 0.05)(Dm, H, Dh) * Dm ** (-0.5)), 'Wk': _w((lambda *s: _rng.normal(s) * 0.05)(Dm, H, Dh) * Dm ** (-0.5)), 'Wv': _w((lambda *s: _rng.normal(s) * 0.05)(Dm, H, Dh) * Dm ** (-0.5)), 'Wo': _w((lambda *s: _rng.normal(s) * 0.05)(H, Dh, Dm) * (H * Dh) ** (-0.5)), 'seg_len': seg}
    _B_in = _B_setup()
    return {'A_x': _A_in['x'], 'A_wqkv': _A_in['wqkv'], 'A_wo': _A_in['wo'], 'B_x': _B_in['x'], 'B_mem0': _B_in['mem0'], 'B_Wq': _B_in['Wq'], 'B_Wk': _B_in['Wk'], 'B_Wv': _B_in['Wv'], 'B_Wo': _B_in['Wo'], 'B_seg_len': _B_in['seg_len']}

def reference(A_x, A_wqkv, A_wo, B_x, B_mem0, B_Wq, B_Wk, B_Wv, B_Wo, B_seg_len):

    def _A_ref(x, wqkv, wo):
        B, S, D = x.shape
        H = 32
        Dh = D // H
        W, dil = (8, 2)
        qkv = (lambda x, *d: x.transpose(*d))((x @ wqkv).reshape(B, S, 3, H, Dh), 2, 0, 3, 1, 4)
        q, k, v = (qkv[0], qkv[1], qkv[2])
        scale = Dh ** (-0.5)
        pos = jnp.arange(S)
        off = jnp.arange(W) * dil
        idx = pos[:, None] - off[None, :]
        mask = idx >= 0
        idx_c = jnp.where(mask, idx, 0).reshape(-1)
        kg = k[:, :, idx_c, :].reshape(B, H, S, W, Dh)
        vg = v[:, :, idx_c, :].reshape(B, H, S, W, Dh)
        logits = jnp.einsum('bhsd,bhswd->bhsw', q, kg) * scale
        logits = jnp.where(mask[None, None, :, :], logits, -1000000000.0)
        attn = _softmax(logits, axis=-1)
        o = jnp.einsum('bhsw,bhswd->bhsd', attn, vg)
        return (lambda x, *d: x.transpose(*d))(o, 0, 2, 1, 3).reshape(B, S, D) @ wo

    def _B_ref(x, mem0, Wq, Wk, Wv, Wo, seg_len):
        B, S, Dm = x.shape
        H, Dh = (Wq.shape[1], Wq.shape[2])
        M = mem0.shape[1]
        scale = Dh ** (-0.5)
        n_seg = S // seg_len
        L = M + seg_len
        idx = jnp.arange(L)
        mask = (idx[:, None] < M) | (idx[:, None] >= idx[None, :])
        mem = mem0
        outs = []
        for s in range(n_seg):
            xs = x[:, s * seg_len:(s + 1) * seg_len, :].copy()
            h = jnp.concatenate([mem, xs], axis=1)
            q = jnp.einsum('btd,dhe->bhte', h, Wq)
            k = jnp.einsum('btd,dhe->bhte', h, Wk)
            v = jnp.einsum('btd,dhe->bhte', h, Wv)
            scores = jnp.einsum('bhqe,bhke->bhqk', q, k) * scale
            scores = jnp.where(mask[None, None], scores, -1000000000.0)
            p = _softmax(scores, axis=-1)
            o = jnp.einsum('bhqk,bhke->bhqe', p, v)
            o = jnp.einsum('bhte,hed->btd', o, Wo)
            mem = o[:, :M, :].copy()
            outs.append(o[:, M:, :])
        return jnp.concatenate(outs, axis=1)
    a = _A_ref(A_x, A_wqkv, A_wo)
    b = _B_ref(B_x, B_mem0, B_Wq, B_Wk, B_Wv, B_Wo, B_seg_len)
    return jnp.concatenate([a, b], axis=-1)
```

```python
import jax
import jax.numpy as jnp
from jax import lax
import jax.experimental.pallas as pl
import jax.experimental.pallas.tpu as pltpu

F32 = jnp.float32
BF16 = jnp.bfloat16
U32 = jnp.uint32

LANES = 128
A_HEADS = 32
A_WIN = 8
A_DIL = 2
A_CHUNK = 128
A_HALO = 16
NEG = -1000000000.0


def _nn(a, b):
    return lax.dot_general(a, b, (((1,), (0,)), ((), ())), preferred_element_type=F32)


def _nt(a, b):
    return lax.dot_general(a, b, (((1,), (1,)), ((), ())), preferred_element_type=F32)


def _build(S, D, M, H, Dh, seg):
    nt_d = D // LANES
    a_dh = D // A_HEADS
    n_chunk = S // A_CHUNK
    n_pair = H // 2
    PW = 2 * Dh
    L = M + seg
    n_seg = S // seg
    assert D % LANES == 0 and 4 * A_HEADS == LANES and a_dh == 4 * nt_d
    assert PW == 3 * LANES and n_pair == n_chunk and n_chunk % 2 == 0
    assert M % 8 == 0 and seg % 16 == 0 and 2 * L <= LANES
    a_scale = a_dh ** -0.5
    b_scale = Dh ** -0.5

    def kernel(ax_hbm, awqkv_hbm, awo_hbm, bx_hbm, mem_hbm, wq_hbm, wk_hbm, wv_hbm, wo_hbm,
               out_hbm,
               ax, awqkv_raw, awo_raw, aw_t, awp, awo_t, awop,
               q0, q1, k0, k1, v0, v1, o0, o1, a_out,
               bx, mem0, wraw, wo_raw, wqkv, wo, h_ref, b_out,
               sem_in, sem_w, sem_wo, sem_out):
        cp_awqkv = pltpu.make_async_copy(awqkv_hbm, awqkv_raw, sem_in.at[0])
        cp_ax = pltpu.make_async_copy(ax_hbm, ax, sem_in.at[1])
        cp_awo = pltpu.make_async_copy(awo_hbm, awo_raw, sem_in.at[2])
        cp_bx = pltpu.make_async_copy(bx_hbm, bx, sem_in.at[3])
        cp_mem = pltpu.make_async_copy(mem_hbm, mem0, sem_in.at[4])
        cp_aout = pltpu.make_async_copy(a_out, out_hbm.at[:, pl.ds(0, D)], sem_out.at[0])
        cp_bout = pltpu.make_async_copy(b_out, out_hbm.at[:, pl.ds(D, D)], sem_out.at[1])

        def cp_w(j, g):
            src = (wq_hbm, wk_hbm, wv_hbm)[j]
            return pltpu.make_async_copy(src.at[g], wraw.at[j, g], sem_w.at[j * n_pair + g])

        cp_wo = pltpu.make_async_copy(wo_hbm, wo_raw, sem_wo.at[0])

        cp_awqkv.start()
        cp_ax.start()
        cp_awo.start()

        def reorder(src, dst, base):
            for j in range(a_dh // 2):
                for t in range(nt_d):
                    x = src[t, pl.ds(base + j, A_HEADS, stride=a_dh // 2), :]
                    even = pltpu.bitcast(x << 16, F32)
                    odd = pltpu.bitcast((x >> 16) << 16, F32)
                    y = jnp.concatenate([even, odd], axis=0).astype(BF16)
                    dst[pl.ds(base + A_HEADS * j, A_HEADS), t * LANES:(t + 1) * LANES] = pltpu.bitcast(y, U32)

        cp_awqkv.wait()
        for t in range(nt_d):
            aw_t[t] = pltpu.bitcast(awqkv_raw[t * LANES:(t + 1) * LANES, :].T, U32)
        for p in range(3):
            reorder(aw_t, awp, p * D // 2)
        cp_ax.wait()
        cp_awo.wait()
        for g in range(n_pair):
            for j in range(3):
                cp_w(j, g).start()
        cp_wo.start()
        cp_mem.start()
        cp_bx.start()
        for t in range(nt_d):
            awo_t[t] = pltpu.bitcast(awo_raw[:, t * LANES:(t + 1) * LANES], U32)
        reorder(awo_t, awop, 0)

        def a_proj(c, bufs, n):
            q, k, v = bufs
            x = ax[pl.ds(pl.multiple_of(c * A_CHUNK, A_CHUNK), A_CHUNK), :]
            w = pltpu.bitcast(awp[n * (LANES // 2):(n + 1) * (LANES // 2), :], BF16)
            r = _nt(x, w)
            part, t = divmod(n, nt_d)
            if part == 0:
                q[t] = r
            else:
                (k, v)[part - 1][t, A_HALO:, :] = r

        def a_attn(c, bufs, o, r):
            q, k, v = bufs
            qs = [q[t, 8 * r:8 * r + 8, :] for t in range(nt_d)]
            logits = []
            for w in range(A_WIN):
                off = A_HALO + 8 * r - A_DIL * w
                s = qs[0] * k[0, off:off + 8, :]
                for t in range(1, nt_d):
                    s = s + qs[t] * k[t, off:off + 8, :]
                s = s + pltpu.roll(s, 2 * A_HEADS, 1)
                s = s + pltpu.roll(s, A_HEADS, 1)
                s = s * a_scale
                if 8 * r < A_DIL * w:
                    pos = c * A_CHUNK + 8 * r + lax.broadcasted_iota(jnp.int32, (8, LANES), 0)
                    s = jnp.where(pos >= A_DIL * w, s, NEG)
                logits.append(s)
            m = logits[0]
            for s in logits[1:]:
                m = jnp.maximum(m, s)
            es = [jnp.exp(s - m) for s in logits]
            den = es[0]
            for e in es[1:]:
                den = den + e
            inv = 1.0 / den
            ps = [e * inv for e in es]
            for t in range(nt_d):
                acc = None
                for w in range(A_WIN):
                    off = A_HALO + 8 * r - A_DIL * w
                    term = ps[w] * v[t, off:off + 8, :]
                    acc = term if acc is None else acc + term
                o[8 * r:8 * r + 8, t * LANES:(t + 1) * LANES] = acc

        def a_oproj(c, o, t):
            w = pltpu.bitcast(awop[:, t * LANES:(t + 1) * LANES], BF16)
            r = _nn(o[...], w)
            a_out[pl.ds(pl.multiple_of(c * A_CHUNK, A_CHUNK), A_CHUNK), t * LANES:(t + 1) * LANES] = r.astype(BF16)

        def b_prep(g, i):
            j, t = divmod(i, PW // LANES)
            blk = wraw[j, g, t * LANES:(t + 1) * LANES, :]
            wqkv[g, :, i * LANES:(i + 1) * LANES] = pltpu.bitcast(blk.T, U32)

        n_proj = 3 * nt_d
        n_grp = A_CHUNK // 8

        def a_step(c, cur, nxt, o_cur, o_prev, do_proj, do_oproj):
            for j in range(3):
                cp_w(j, c).wait()
            if do_proj:
                for src, dst in ((cur[1], nxt[1]), (cur[2], nxt[2])):
                    for t in range(nt_d):
                        dst[t, 0:A_HALO, :] = src[t, A_CHUNK:A_CHUNK + A_HALO, :]
            mxu = []
            if do_oproj:
                mxu += [(lambda t=t: a_oproj(c - 1, o_prev, t)) for t in range(nt_d)]
            if do_proj:
                mxu += [(lambda n=n: a_proj(c + 1, nxt, n)) for n in range(n_proj)]
            done = 0
            for r in range(n_grp):
                upto = (r + 1) * len(mxu) // n_grp
                for f in mxu[done:upto]:
                    f()
                done = upto
                a_attn(c, cur, o_cur, r)
                if r < 9:
                    b_prep(c, r)

        buf0 = (q0, k0, v0)
        buf1 = (q1, k1, v1)
        for n in range(n_proj):
            a_proj(0, buf0, n)
        for t in range(nt_d):
            k0[t, 0:A_HALO, :] = jnp.broadcast_to(k0[t, A_HALO:A_HALO + 1, :], (A_HALO, LANES))
            v0[t, 0:A_HALO, :] = jnp.broadcast_to(v0[t, A_HALO:A_HALO + 1, :], (A_HALO, LANES))
        a_step(0, buf0, buf1, o0, o1, True, False)

        def a_body(i, carry):
            a_step(2 * i + 1, buf1, buf0, o1, o0, True, True)
            a_step(2 * i + 2, buf0, buf1, o0, o1, True, True)
            return carry

        lax.fori_loop(0, n_chunk // 2 - 1, a_body, 0)
        a_step(n_chunk - 1, buf1, buf0, o1, o0, False, True)
        for t in range(nt_d):
            a_oproj(n_chunk - 1, o1, t)
        cp_aout.start()

        cp_wo.wait()

        def retile(g, carry):
            wo[g] = pltpu.bitcast(wo_raw[g], U32)
            return carry

        lax.fori_loop(0, n_pair, retile, 0)
        cp_mem.wait()
        cp_bx.wait()
        h_ref[0:M, :] = mem0[...].astype(F32)

        def b_body(s, carry):
            r0 = pl.multiple_of(s * seg, seg)
            h_ref[M:L, :] = bx[pl.ds(r0, seg), :].astype(F32)
            low = lax.broadcasted_iota(jnp.int32, (L, LANES), 1) < Dh - LANES
            col = lax.broadcasted_iota(jnp.int32, (L, 2 * L), 1)
            row = lax.broadcasted_iota(jnp.int32, (L, 2 * L), 0)
            first = col < L
            allow = (row < M) | (row >= jnp.where(first, col, col - L))
            zero = jnp.zeros((L, LANES), F32)

            def blockdiag(x):
                t0, t1, t2 = x[:, 0:LANES], x[:, LANES:2 * LANES], x[:, 2 * LANES:3 * LANES]
                top = jnp.concatenate([t0, jnp.where(low, t1, 0.0), zero], axis=1)
                bot = jnp.concatenate([zero, jnp.where(low, 0.0, t1), t2], axis=1)
                return jnp.concatenate([top, bot], axis=0).astype(BF16)

            st = {}
            acc = []

            def proj(g):
                r = _nn(h_ref[...], pltpu.bitcast(wqkv[g], BF16))
                st[g] = dict(q=r[:, 0:PW], k=blockdiag(r[:, PW:2 * PW]), v=blockdiag(r[:, 2 * PW:3 * PW]))

            def scores(g):
                d = st[g]
                sc = jnp.where(allow, _nt(d['q'], d['k']) * b_scale, NEG)
                m0 = jnp.max(jnp.where(first, sc, -jnp.inf), axis=1, keepdims=True)
                m1 = jnp.max(jnp.where(first, -jnp.inf, sc), axis=1, keepdims=True)
                e = jnp.exp(sc - jnp.where(first, m0, m1))
                l0 = jnp.sum(jnp.where(first, e, 0.0), axis=1, keepdims=True)
                l1 = jnp.sum(jnp.where(first, 0.0, e), axis=1, keepdims=True)
                d['p'] = e / jnp.where(first, l0, l1)

            def mix(g):
                d = st[g]
                d['o'] = _nn(d['p'], d['v'])

            def oproj(g):
                r = _nn(st.pop(g)['o'], pltpu.bitcast(wo[g], BF16))
                acc[:] = [r if not acc else acc[0] + r]

            stages = ((proj, 0), (scores, 1), (mix, 3), (oproj, 4))
            for t in range(n_pair + stages[-1][1]):
                for fn, lag in stages:
                    if 0 <= t - lag < n_pair:
                        fn(t - lag)
            out = acc[0]
            h_ref[0:M, :] = out[0:M].astype(BF16).astype(F32)
            b_out[pl.ds(r0, seg), :] = out[M:L].astype(BF16)
            return carry

        lax.fori_loop(0, n_seg, b_body, 0)
        cp_bout.start()
        cp_aout.wait()
        cp_bout.wait()

    qbuf = pltpu.VMEM((nt_d, A_CHUNK, LANES), F32)
    kbuf = pltpu.VMEM((nt_d, A_HALO + A_CHUNK, LANES), F32)
    obuf = pltpu.VMEM((A_CHUNK, D), F32)
    scratch = [
        pltpu.VMEM((S, D), BF16),
        pltpu.VMEM((D, 3 * D), BF16),
        pltpu.VMEM((D, D), BF16),
        pltpu.VMEM((nt_d, 3 * D // 2, LANES), U32),
        pltpu.VMEM((3 * D // 2, D), U32),
        pltpu.VMEM((nt_d, D // 2, LANES), U32),
        pltpu.VMEM((D // 2, D), U32),
        qbuf, qbuf, kbuf, kbuf, kbuf, kbuf, obuf, obuf,
        pltpu.VMEM((S, D), BF16),
        pltpu.VMEM((S, D), BF16),
        pltpu.VMEM((M, D), BF16),
        pltpu.VMEM((3, n_pair, PW, D), BF16),
        pltpu.VMEM((n_pair, PW, D), BF16),
        pltpu.VMEM((n_pair, D // 2, 3 * PW), U32),
        pltpu.VMEM((n_pair, PW // 2, D), U32),
        pltpu.VMEM((L, D), F32),
        pltpu.VMEM((S, D), BF16),
        pltpu.SemaphoreType.DMA((5,)),
        pltpu.SemaphoreType.DMA((3 * n_pair,)),
        pltpu.SemaphoreType.DMA((1,)),
        pltpu.SemaphoreType.DMA((2,)),
    ]
    return pl.pallas_call(
        kernel,
        out_shape=jax.ShapeDtypeStruct((S, 2 * D), BF16),
        in_specs=[pl.BlockSpec(memory_space=pl.ANY)] * 9,
        out_specs=pl.BlockSpec(memory_space=pl.ANY),
        scratch_shapes=scratch,
        compiler_params=pltpu.CompilerParams(vmem_limit_bytes=110 * 1024 * 1024),
    )


def pallas_concat_heads__sliding_local_dilated__memory_aug_recurrent_mem_tr__prompt_kernel(
    A_x, A_wqkv, A_wo, B_x, B_mem0, B_Wq, B_Wk, B_Wv, B_Wo, B_seg_len,
):
    batch, S, D = B_x.shape
    M = B_mem0.shape[1]
    _, H, Dh = B_Wq.shape
    assert batch == 1 and A_x.shape == B_x.shape

    def pairs(w):
        return jnp.transpose(w, (1, 2, 0)).reshape(H // 2, 2 * Dh, D)

    out = _build(S, D, M, H, Dh, int(B_seg_len))(
        A_x.reshape(S, D), A_wqkv, A_wo, B_x.reshape(S, D), B_mem0.reshape(M, D),
        pairs(B_Wq), pairs(B_Wk), pairs(B_Wv), B_Wo.reshape(H // 2, 2 * Dh, D))
    return out.reshape(1, S, 2 * D)
```

```python
import jax
import jax.numpy as jnp
from jax import lax
import jax.experimental.pallas as pl
import jax.experimental.pallas.tpu as pltpu

F32 = jnp.float32
BF16 = jnp.bfloat16
U32 = jnp.uint32

LANES = 128
A_HEADS = 32
A_WIN = 8
A_DIL = 2
A_CHUNK = 128
A_HALO = 16
NEG = -1000000000.0


def _nn(a, b):
    return lax.dot_general(a, b, (((1,), (0,)), ((), ())), preferred_element_type=F32)


def _nt(a, b):
    return lax.dot_general(a, b, (((1,), (1,)), ((), ())), preferred_element_type=F32)


def _build(S, D, M, H, Dh, seg):
    nt_d = D // LANES
    a_dh = D // A_HEADS
    n_chunk = S // A_CHUNK
    n_pair = H // 2
    PW = 2 * Dh
    L = M + seg
    n_seg = S // seg
    assert D % LANES == 0 and 4 * A_HEADS == LANES and a_dh == 4 * nt_d
    assert PW == 3 * LANES and n_pair == n_chunk and n_chunk % 2 == 0
    assert M % 8 == 0 and seg % 16 == 0 and 2 * L <= LANES
    a_scale = a_dh ** -0.5
    b_scale = Dh ** -0.5

    def kernel(ax_hbm, awqkv_hbm, awo_hbm, bx_hbm, mem_hbm, wq_hbm, wk_hbm, wv_hbm, wo_hbm,
               out_hbm,
               ax, awqkv_raw, awo_raw, aw_t, awp, awo_t, awop,
               q0, q1, k0, k1, v0, v1, o0, o1, a_out,
               bx, mem0, wraw, wo_raw, wqkv, wo, h_ref, b_out,
               sem_in, sem_w, sem_wo, sem_out):
        cp_awqkv = pltpu.make_async_copy(awqkv_hbm, awqkv_raw, sem_in.at[0])
        cp_ax = pltpu.make_async_copy(ax_hbm, ax, sem_in.at[1])
        cp_awo = pltpu.make_async_copy(awo_hbm, awo_raw, sem_in.at[2])
        cp_bx = pltpu.make_async_copy(bx_hbm, bx, sem_in.at[3])
        cp_mem = pltpu.make_async_copy(mem_hbm, mem0, sem_in.at[4])
        cp_aout = pltpu.make_async_copy(a_out, out_hbm.at[:, pl.ds(0, D)], sem_out.at[0])
        cp_bout = pltpu.make_async_copy(b_out, out_hbm.at[:, pl.ds(D, D)], sem_out.at[1])

        def cp_w(j, g):
            src = (wq_hbm, wk_hbm, wv_hbm)[j]
            return pltpu.make_async_copy(src.at[g], wraw.at[j, g], sem_w.at[j * n_pair + g])

        cp_wo = pltpu.make_async_copy(wo_hbm, wo_raw, sem_wo.at[0])

        cp_awqkv.start()
        cp_ax.start()
        cp_awo.start()

        def reorder(src, dst, base):
            for j in range(a_dh // 2):
                for t in range(nt_d):
                    x = src[t, pl.ds(base + j, A_HEADS, stride=a_dh // 2), :]
                    even = pltpu.bitcast(x << 16, F32)
                    odd = pltpu.bitcast((x >> 16) << 16, F32)
                    y = jnp.concatenate([even, odd], axis=0).astype(BF16)
                    dst[pl.ds(base + A_HEADS * j, A_HEADS), t * LANES:(t + 1) * LANES] = pltpu.bitcast(y, U32)

        cp_awqkv.wait()
        for t in range(nt_d):
            aw_t[t] = pltpu.bitcast(awqkv_raw[t * LANES:(t + 1) * LANES, :].T, U32)
        for p in range(3):
            reorder(aw_t, awp, p * D // 2)
        cp_ax.wait()
        cp_awo.wait()
        for g in range(n_pair):
            for j in range(3):
                cp_w(j, g).start()
        cp_wo.start()
        cp_mem.start()
        cp_bx.start()
        for t in range(nt_d):
            awo_t[t] = pltpu.bitcast(awo_raw[:, t * LANES:(t + 1) * LANES], U32)
        reorder(awo_t, awop, 0)

        def a_proj(c, bufs, n):
            q, k, v = bufs
            x = ax[pl.ds(pl.multiple_of(c * A_CHUNK, A_CHUNK), A_CHUNK), :]
            w = pltpu.bitcast(awp[n * (LANES // 2):(n + 1) * (LANES // 2), :], BF16)
            r = _nt(x, w)
            part, t = divmod(n, nt_d)
            if part == 0:
                q[t] = r
            else:
                (k, v)[part - 1][t, A_HALO:, :] = r

        def a_dots(bufs, r):
            q, k, _ = bufs
            qs = [q[t, 8 * r:8 * r + 8, :] for t in range(nt_d)]
            part = []
            for w in range(A_WIN):
                off = A_HALO + 8 * r - A_DIL * w
                s = qs[0] * k[0, off:off + 8, :]
                for t in range(1, nt_d):
                    s = s + qs[t] * k[t, off:off + 8, :]
                part.append(s + pltpu.roll(s, 2 * A_HEADS, 1))
            return part

        def a_fold(part):
            return [s + pltpu.roll(s, A_HEADS, 1) for s in part]

        def a_mix(c, bufs, o, r, dots):
            v = bufs[2]
            logits = []
            for w, s in enumerate(dots):
                s = s * a_scale
                if 8 * r < A_DIL * w:
                    pos = c * A_CHUNK + 8 * r + lax.broadcasted_iota(jnp.int32, (8, LANES), 0)
                    s = jnp.where(pos >= A_DIL * w, s, NEG)
                logits.append(s)
            m = logits[0]
            for s in logits[1:]:
                m = jnp.maximum(m, s)
            es = [jnp.exp(s - m) for s in logits]
            den = es[0]
            for e in es[1:]:
                den = den + e
            inv = 1.0 / den
            ps = [e * inv for e in es]
            for t in range(nt_d):
                acc = None
                for w in range(A_WIN):
                    off = A_HALO + 8 * r - A_DIL * w
                    term = ps[w] * v[t, off:off + 8, :]
                    acc = term if acc is None else acc + term
                o[8 * r:8 * r + 8, t * LANES:(t + 1) * LANES] = acc

        def a_oproj(c, o, t):
            w = pltpu.bitcast(awop[:, t * LANES:(t + 1) * LANES], BF16)
            r = _nn(o[...], w)
            a_out[pl.ds(pl.multiple_of(c * A_CHUNK, A_CHUNK), A_CHUNK), t * LANES:(t + 1) * LANES] = r.astype(BF16)

        def b_prep(g, i):
            j, t = divmod(i, PW // LANES)
            blk = wraw[j, g, t * LANES:(t + 1) * LANES, :]
            wqkv[g, :, i * LANES:(i + 1) * LANES] = pltpu.bitcast(blk.T, U32)

        n_proj = 3 * nt_d
        n_grp = A_CHUNK // 8

        def a_step(c, cur, nxt, o_cur, o_prev, do_proj, do_oproj):
            for j in range(3):
                cp_w(j, c).wait()
            if do_proj:
                for src, dst in ((cur[1], nxt[1]), (cur[2], nxt[2])):
                    for t in range(nt_d):
                        dst[t, 0:A_HALO, :] = src[t, A_CHUNK:A_CHUNK + A_HALO, :]
            mxu = []
            if do_oproj:
                mxu += [(lambda t=t: a_oproj(c - 1, o_prev, t)) for t in range(nt_d)]
            if do_proj:
                mxu += [(lambda n=n: a_proj(c + 1, nxt, n)) for n in range(n_proj)]
            done = 0
            st = {}
            n_slot = n_grp + 2
            for r in range(n_slot):
                upto = (r + 1) * len(mxu) // n_slot
                for f in mxu[done:upto]:
                    f()
                done = upto
                if r < n_grp:
                    st[r] = a_dots(cur, r)
                if 0 <= r - 1 < n_grp:
                    st[r - 1] = a_fold(st[r - 1])
                if r % 2 == 0:
                    b_prep(c, r // 2)
                if 0 <= r - 2 < n_grp:
                    a_mix(c, cur, o_cur, r - 2, st.pop(r - 2))

        buf0 = (q0, k0, v0)
        buf1 = (q1, k1, v1)
        for n in range(n_proj):
            a_proj(0, buf0, n)
        for t in range(nt_d):
            k0[t, 0:A_HALO, :] = jnp.broadcast_to(k0[t, A_HALO:A_HALO + 1, :], (A_HALO, LANES))
            v0[t, 0:A_HALO, :] = jnp.broadcast_to(v0[t, A_HALO:A_HALO + 1, :], (A_HALO, LANES))
        a_step(0, buf0, buf1, o0, o1, True, False)

        def a_body(i, carry):
            a_step(2 * i + 1, buf1, buf0, o1, o0, True, True)
            a_step(2 * i + 2, buf0, buf1, o0, o1, True, True)
            return carry

        lax.fori_loop(0, n_chunk // 2 - 1, a_body, 0)
        a_step(n_chunk - 1, buf1, buf0, o1, o0, False, True)
        for t in range(nt_d):
            a_oproj(n_chunk - 1, o1, t)
        cp_aout.start()

        cp_wo.wait()

        def retile(g, carry):
            wo[g] = pltpu.bitcast(wo_raw[g], U32)
            return carry

        lax.fori_loop(0, n_pair, retile, 0)
        cp_mem.wait()
        cp_bx.wait()
        h_ref[0:M, :] = mem0[...].astype(F32)

        def b_body(s, carry):
            r0 = pl.multiple_of(s * seg, seg)
            h_ref[M:L, :] = bx[pl.ds(r0, seg), :].astype(F32)
            low = lax.broadcasted_iota(jnp.int32, (L, LANES), 1) < Dh - LANES
            col = lax.broadcasted_iota(jnp.int32, (L, 2 * L), 1)
            row = lax.broadcasted_iota(jnp.int32, (L, 2 * L), 0)
            first = col < L
            allow = (row < M) | (row >= jnp.where(first, col, col - L))
            zero = jnp.zeros((L, LANES), F32)

            def blockdiag(x):
                t0, t1, t2 = x[:, 0:LANES], x[:, LANES:2 * LANES], x[:, 2 * LANES:3 * LANES]
                top = jnp.concatenate([t0, jnp.where(low, t1, 0.0), zero], axis=1)
                bot = jnp.concatenate([zero, jnp.where(low, 0.0, t1), t2], axis=1)
                return jnp.concatenate([top, bot], axis=0).astype(BF16)

            st = {}
            acc = []

            def proj(g):
                r = _nn(h_ref[...], pltpu.bitcast(wqkv[g], BF16))
                st[g] = dict(q=r[:, 0:PW], k=blockdiag(r[:, PW:2 * PW]), v=blockdiag(r[:, 2 * PW:3 * PW]))

            def scores(g):
                d = st[g]
                sc = jnp.where(allow, _nt(d['q'], d['k']) * b_scale, NEG)
                m0 = jnp.max(jnp.where(first, sc, -jnp.inf), axis=1, keepdims=True)
                m1 = jnp.max(jnp.where(first, -jnp.inf, sc), axis=1, keepdims=True)
                e = jnp.exp(sc - jnp.where(first, m0, m1))
                l0 = jnp.sum(jnp.where(first, e, 0.0), axis=1, keepdims=True)
                l1 = jnp.sum(jnp.where(first, 0.0, e), axis=1, keepdims=True)
                d['p'] = e / jnp.where(first, l0, l1)

            def mix(g):
                d = st[g]
                d['o'] = _nn(d['p'], d['v'])

            def oproj(g):
                r = _nn(st.pop(g)['o'], pltpu.bitcast(wo[g], BF16))
                acc[:] = [r if not acc else acc[0] + r]

            stages = ((proj, 0), (scores, 1), (mix, 3), (oproj, 4))
            for t in range(n_pair + stages[-1][1]):
                for fn, lag in stages:
                    if 0 <= t - lag < n_pair:
                        fn(t - lag)
            out = acc[0]
            h_ref[0:M, :] = out[0:M].astype(BF16).astype(F32)
            b_out[pl.ds(r0, seg), :] = out[M:L].astype(BF16)
            return carry

        lax.fori_loop(0, n_seg, b_body, 0)
        cp_bout.start()
        cp_aout.wait()
        cp_bout.wait()

    qbuf = pltpu.VMEM((nt_d, A_CHUNK, LANES), F32)
    kbuf = pltpu.VMEM((nt_d, A_HALO + A_CHUNK, LANES), F32)
    obuf = pltpu.VMEM((A_CHUNK, D), F32)
    scratch = [
        pltpu.VMEM((S, D), BF16),
        pltpu.VMEM((D, 3 * D), BF16),
        pltpu.VMEM((D, D), BF16),
        pltpu.VMEM((nt_d, 3 * D // 2, LANES), U32),
        pltpu.VMEM((3 * D // 2, D), U32),
        pltpu.VMEM((nt_d, D // 2, LANES), U32),
        pltpu.VMEM((D // 2, D), U32),
        qbuf, qbuf, kbuf, kbuf, kbuf, kbuf, obuf, obuf,
        pltpu.VMEM((S, D), BF16),
        pltpu.VMEM((S, D), BF16),
        pltpu.VMEM((M, D), BF16),
        pltpu.VMEM((3, n_pair, PW, D), BF16),
        pltpu.VMEM((n_pair, PW, D), BF16),
        pltpu.VMEM((n_pair, D // 2, 3 * PW), U32),
        pltpu.VMEM((n_pair, PW // 2, D), U32),
        pltpu.VMEM((L, D), F32),
        pltpu.VMEM((S, D), BF16),
        pltpu.SemaphoreType.DMA((5,)),
        pltpu.SemaphoreType.DMA((3 * n_pair,)),
        pltpu.SemaphoreType.DMA((1,)),
        pltpu.SemaphoreType.DMA((2,)),
    ]
    return pl.pallas_call(
        kernel,
        out_shape=jax.ShapeDtypeStruct((S, 2 * D), BF16),
        in_specs=[pl.BlockSpec(memory_space=pl.ANY)] * 9,
        out_specs=pl.BlockSpec(memory_space=pl.ANY),
        scratch_shapes=scratch,
        compiler_params=pltpu.CompilerParams(vmem_limit_bytes=110 * 1024 * 1024),
    )


def pallas_concat_heads__sliding_local_dilated__memory_aug_recurrent_mem_tr__prompt_kernel(
    A_x, A_wqkv, A_wo, B_x, B_mem0, B_Wq, B_Wk, B_Wv, B_Wo, B_seg_len,
):
    batch, S, D = B_x.shape
    M = B_mem0.shape[1]
    _, H, Dh = B_Wq.shape
    assert batch == 1 and A_x.shape == B_x.shape

    def pairs(w):
        return jnp.transpose(w, (1, 2, 0)).reshape(H // 2, 2 * Dh, D)

    out = _build(S, D, M, H, Dh, int(B_seg_len))(
        A_x.reshape(S, D), A_wqkv, A_wo, B_x.reshape(S, D), B_mem0.reshape(M, D),
        pairs(B_Wq), pairs(B_Wk), pairs(B_Wv), B_Wo.reshape(H // 2, 2 * Dh, D))
    return out.reshape(1, S, 2 * D)
```

```python
import jax
import jax.numpy as jnp
from jax import lax
import jax.experimental.pallas as pl
import jax.experimental.pallas.tpu as pltpu

F32 = jnp.float32
BF16 = jnp.bfloat16
U32 = jnp.uint32

LANES = 128
A_HEADS = 32
A_WIN = 8
A_DIL = 2
A_CHUNK = 128
A_HALO = 16
B_UNROLL = 3
WO_GROUP = 4
NEG = -1000000000.0


def _nn(a, b):
    return lax.dot_general(a, b, (((1,), (0,)), ((), ())), preferred_element_type=F32)


def _nt(a, b):
    return lax.dot_general(a, b, (((1,), (1,)), ((), ())), preferred_element_type=F32)


def _build(S, D, M, H, Dh, seg):
    nt_d = D // LANES
    a_dh = D // A_HEADS
    n_chunk = S // A_CHUNK
    n_pair = H // 2
    PW = 2 * Dh
    L = M + seg
    n_seg = S // seg
    assert D % LANES == 0 and 4 * A_HEADS == LANES and a_dh == 4 * nt_d
    assert PW == 3 * LANES and n_pair == n_chunk and n_chunk % 2 == 0
    assert M % 8 == 0 and seg % 16 == 0 and 2 * L <= LANES
    assert (n_seg - 1) % B_UNROLL == 0 and n_pair % WO_GROUP == 0
    sem_aw = 4
    sem_ax = sem_aw + nt_d
    sem_w = sem_ax + n_chunk
    sem_wo = sem_w + 3 * n_pair
    a_scale = a_dh ** -0.5
    b_scale = Dh ** -0.5

    def kernel(ax_hbm, awqkv_hbm, awo_hbm, bx_hbm, mem_hbm, wq_hbm, wk_hbm, wv_hbm, wo_hbm,
               out_hbm,
               ax, awqkv_raw, awo_raw, aw_t, awp, awo_t, awop,
               q0, q1, k0, k1, v0, v1, o0, o1, a_out,
               bx, mem0, wraw, wo_raw, wqkv, wo, h0, h1, h2, h3, b_out,
               sem_in, sem_out):
        cp_awo = pltpu.make_async_copy(awo_hbm, awo_raw, sem_in.at[0])
        cp_mem = pltpu.make_async_copy(mem_hbm, mem0, sem_in.at[1])
        cp_bx0 = pltpu.make_async_copy(bx_hbm.at[pl.ds(0, seg)], bx.at[pl.ds(0, seg)], sem_in.at[2])
        cp_bx1 = pltpu.make_async_copy(bx_hbm.at[pl.ds(seg, S - seg)], bx.at[pl.ds(seg, S - seg)], sem_in.at[3])
        cp_aout = pltpu.make_async_copy(a_out, out_hbm.at[:, pl.ds(0, D)], sem_out.at[0])

        def cp_awqkv(t):
            rows = pl.ds(t * LANES, LANES)
            return pltpu.make_async_copy(awqkv_hbm.at[rows], awqkv_raw.at[rows], sem_in.at[sem_aw + t])

        def cp_ax(c):
            rows = pl.ds(pl.multiple_of(c * A_CHUNK, A_CHUNK), A_CHUNK)
            return pltpu.make_async_copy(ax_hbm.at[rows], ax.at[rows], sem_in.at[sem_ax + c])

        def cp_w(j, g):
            src = (wq_hbm, wk_hbm, wv_hbm)[j]
            return pltpu.make_async_copy(src.at[g], wraw.at[j, g], sem_in.at[sem_w + j * n_pair + g])

        def cp_wo(g):
            return pltpu.make_async_copy(wo_hbm.at[g], wo_raw.at[g], sem_in.at[sem_wo + g])

        def cp_bout(s0, n, sem):
            rows = pl.ds(pl.multiple_of(s0 * seg, seg), n * seg)
            return pltpu.make_async_copy(b_out.at[rows], out_hbm.at[rows, pl.ds(D, D)], sem)

        for t in range(nt_d):
            cp_awqkv(t).start()
        cp_ax(0).start()
        cp_ax(1).start()
        cp_awo.start()
        for g in range(n_pair):
            if g + 2 < n_chunk:
                cp_ax(g + 2).start()
            for j in range(3):
                cp_w(j, g).start()
        cp_mem.start()
        cp_bx0.start()
        for g in range(n_pair):
            cp_wo(g).start()
        cp_bx1.start()

        def reorder(src, dst, base):
            for j in range(a_dh // 2):
                for t in range(nt_d):
                    x = src[t, pl.ds(base + j, A_HEADS, stride=a_dh // 2), :]
                    even = pltpu.bitcast(x << 16, F32)
                    odd = pltpu.bitcast((x >> 16) << 16, F32)
                    y = jnp.concatenate([even, odd], axis=0).astype(BF16)
                    dst[pl.ds(base + A_HEADS * j, A_HEADS), t * LANES:(t + 1) * LANES] = pltpu.bitcast(y, U32)

        for t in range(nt_d):
            cp_awqkv(t).wait()
            aw_t[t] = pltpu.bitcast(awqkv_raw[t * LANES:(t + 1) * LANES, :].T, U32)
        for p in range(3):
            reorder(aw_t, awp, p * D // 2)

        def a_proj(c, bufs, n):
            q, k, v = bufs
            x = ax[pl.ds(pl.multiple_of(c * A_CHUNK, A_CHUNK), A_CHUNK), :]
            w = pltpu.bitcast(awp[n * (LANES // 2):(n + 1) * (LANES // 2), :], BF16)
            r = _nt(x, w)
            part, t = divmod(n, nt_d)
            if part == 0:
                q[t] = r
            else:
                (k, v)[part - 1][t, A_HALO:, :] = r

        def a_dots(bufs, r):
            q, k, _ = bufs
            qs = [q[t, 8 * r:8 * r + 8, :] for t in range(nt_d)]
            part = []
            for w in range(A_WIN):
                off = A_HALO + 8 * r - A_DIL * w
                s = qs[0] * k[0, off:off + 8, :]
                for t in range(1, nt_d):
                    s = s + qs[t] * k[t, off:off + 8, :]
                part.append(s + pltpu.roll(s, 2 * A_HEADS, 1))
            return part

        def a_fold(part):
            return [s + pltpu.roll(s, A_HEADS, 1) for s in part]

        def a_mix(c, bufs, o, r, dots):
            v = bufs[2]
            logits = []
            for w, s in enumerate(dots):
                s = s * a_scale
                if 8 * r < A_DIL * w:
                    pos = c * A_CHUNK + 8 * r + lax.broadcasted_iota(jnp.int32, (8, LANES), 0)
                    s = jnp.where(pos >= A_DIL * w, s, NEG)
                logits.append(s)
            m = logits[0]
            for s in logits[1:]:
                m = jnp.maximum(m, s)
            es = [jnp.exp(s - m) for s in logits]
            den = es[0]
            for e in es[1:]:
                den = den + e
            inv = 1.0 / den
            ps = [e * inv for e in es]
            for t in range(nt_d):
                acc = None
                for w in range(A_WIN):
                    off = A_HALO + 8 * r - A_DIL * w
                    term = ps[w] * v[t, off:off + 8, :]
                    acc = term if acc is None else acc + term
                o[8 * r:8 * r + 8, t * LANES:(t + 1) * LANES] = acc

        def a_oproj(c, o, t):
            w = pltpu.bitcast(awop[:, t * LANES:(t + 1) * LANES], BF16)
            r = _nn(o[...], w)
            a_out[pl.ds(pl.multiple_of(c * A_CHUNK, A_CHUNK), A_CHUNK), t * LANES:(t + 1) * LANES] = r.astype(BF16)

        def b_prep(g, i):
            j, t = divmod(i, PW // LANES)
            blk = wraw[j, g, t * LANES:(t + 1) * LANES, :]
            wqkv[g, :, i * LANES:(i + 1) * LANES] = pltpu.bitcast(blk.T, U32)

        n_proj = 3 * nt_d
        n_grp = A_CHUNK // 8
        n_slab = 3 * PW // LANES

        def a_step(c, cur, nxt, o_cur, o_prev, do_proj, do_oproj):
            if do_proj:
                cp_ax(c + 1).wait()
            if do_oproj:
                for j in range(3):
                    cp_w(j, c - 1).wait()
            if do_proj:
                for src, dst in ((cur[1], nxt[1]), (cur[2], nxt[2])):
                    for t in range(nt_d):
                        dst[t, 0:A_HALO, :] = src[t, A_CHUNK:A_CHUNK + A_HALO, :]
            mxu = []
            if do_oproj:
                mxu += [(lambda t=t: a_oproj(c - 1, o_prev, t)) for t in range(nt_d)]
            if do_proj:
                mxu += [(lambda n=n: a_proj(c + 1, nxt, n)) for n in range(n_proj)]
            done = 0
            st = {}
            n_slot = n_grp + 2
            for r in range(n_slot):
                upto = (r + 1) * len(mxu) // n_slot
                for f in mxu[done:upto]:
                    f()
                done = upto
                if r < n_grp:
                    st[r] = a_dots(cur, r)
                if 0 <= r - 1 < n_grp:
                    st[r - 1] = a_fold(st[r - 1])
                if do_oproj and r % 2 == 0 and r // 2 < n_slab:
                    b_prep(c - 1, r // 2)
                if 0 <= r - 2 < n_grp:
                    a_mix(c, cur, o_cur, r - 2, st.pop(r - 2))

        buf0 = (q0, k0, v0)
        buf1 = (q1, k1, v1)
        cp_ax(0).wait()
        cp_awo.wait()
        for n in range(n_proj):
            a_proj(0, buf0, n)
        for t in range(nt_d):
            awo_t[t] = pltpu.bitcast(awo_raw[:, t * LANES:(t + 1) * LANES], U32)
        reorder(awo_t, awop, 0)
        for t in range(nt_d):
            k0[t, 0:A_HALO, :] = jnp.broadcast_to(k0[t, A_HALO:A_HALO + 1, :], (A_HALO, LANES))
            v0[t, 0:A_HALO, :] = jnp.broadcast_to(v0[t, A_HALO:A_HALO + 1, :], (A_HALO, LANES))
        a_step(0, buf0, buf1, o0, o1, True, False)

        def a_body(i, carry):
            a_step(2 * i + 1, buf1, buf0, o1, o0, True, True)
            a_step(2 * i + 2, buf0, buf1, o0, o1, True, True)
            return carry

        lax.fori_loop(0, n_chunk // 2 - 1, a_body, 0)
        a_step(n_chunk - 1, buf1, buf0, o1, o0, False, True)
        for j in range(3):
            cp_w(j, n_pair - 1).wait()
        cp_mem.wait()
        cp_bx0.wait()
        for t in range(nt_d):
            a_oproj(n_chunk - 1, o1, t)
        for i in range(n_slab):
            b_prep(n_pair - 1, i)

        def b_step(s, h_ref, h_next, first_step=False, chained=False):
            r0 = pl.multiple_of(s * seg, seg)
            h_ref[M:L, :] = bx[pl.ds(r0, seg), :].astype(F32)
            low = lax.broadcasted_iota(jnp.int32, (L, LANES), 1) < Dh - LANES
            col = lax.broadcasted_iota(jnp.int32, (L, 2 * L), 1)
            row = lax.broadcasted_iota(jnp.int32, (L, 2 * L), 0)
            first = col < L
            allow = (row < M) | (row >= jnp.where(first, col, col - L))
            zero = jnp.zeros((L, LANES), F32)

            def blockdiag(x):
                t0, t1, t2 = x[:, 0:LANES], x[:, LANES:2 * LANES], x[:, 2 * LANES:3 * LANES]
                top = jnp.concatenate([t0, jnp.where(low, t1, 0.0), zero], axis=1)
                bot = jnp.concatenate([zero, jnp.where(low, 0.0, t1), t2], axis=1)
                return jnp.concatenate([top, bot], axis=0).astype(BF16)

            st = {}
            acc = []

            def proj(g):
                if chained and g == 0:
                    r = None
                    for t in range(nt_d):
                        w = pltpu.bitcast(wqkv[g, t * (LANES // 2):(t + 1) * (LANES // 2), :], BF16)
                        part = _nn(h_ref[:, t * LANES:(t + 1) * LANES], w)
                        r = part if r is None else r + part
                else:
                    r = _nn(h_ref[...], pltpu.bitcast(wqkv[g], BF16))
                st[g] = dict(q=r[:, 0:PW], k=blockdiag(r[:, PW:2 * PW]), v=blockdiag(r[:, 2 * PW:3 * PW]))

            def scores(g):
                d = st[g]
                sc = jnp.where(allow, _nt(d['q'], d['k']) * b_scale, NEG)
                m0 = jnp.max(jnp.where(first, sc, -jnp.inf), axis=1, keepdims=True)
                m1 = jnp.max(jnp.where(first, -jnp.inf, sc), axis=1, keepdims=True)
                e = jnp.exp(sc - jnp.where(first, m0, m1))
                l0 = jnp.sum(jnp.where(first, e, 0.0), axis=1, keepdims=True)
                l1 = jnp.sum(jnp.where(first, 0.0, e), axis=1, keepdims=True)
                d['p'] = e / jnp.where(first, l0, l1)

            def mix(g):
                d = st[g]
                d['o'] = _nn(d['p'], d['v'])

            def oproj(g):
                if first_step:
                    if g % WO_GROUP == 0:
                        for i in range(WO_GROUP):
                            cp_wo(g + i).wait()
                    w = wo_raw[g]
                    wo[g] = pltpu.bitcast(w, U32)
                else:
                    w = pltpu.bitcast(wo[g], BF16)
                r = _nn(st.pop(g)['o'], w)
                acc[:] = [r if not acc else acc[0] + r]

            stages = ((proj, 0), (scores, 1), (mix, 4), (oproj, n_pair if first_step else 6))
            for t in range(n_pair + stages[-1][1]):
                for fn, lag in stages:
                    if 0 <= t - lag < n_pair:
                        fn(t - lag)
            for t in range(nt_d):
                cols = slice(t * LANES, (t + 1) * LANES)
                h_next[0:M, cols] = acc[0][0:M, cols].astype(BF16).astype(F32)
            b_out[pl.ds(r0, seg), :] = acc[0][M:L].astype(BF16)

        hs = (h1, h2, h3)
        h0[0:M, :] = mem0[...].astype(F32)
        b_step(0, h0, hs[0], first_step=True)
        cp_bx1.wait()
        cp_aout.start()
        cp_bout(0, 1, sem_out.at[1]).start()

        def b_body(i, carry):
            s0 = 1 + B_UNROLL * i
            for u in range(B_UNROLL):
                b_step(s0 + u, hs[u], hs[(u + 1) % B_UNROLL], chained=u > 0)

            @pl.when(i > 0)
            def _():
                cp_bout(s0 - B_UNROLL, B_UNROLL, sem_out.at[2]).wait()

            cp_bout(s0, B_UNROLL, sem_out.at[2]).start()
            return carry

        lax.fori_loop(0, (n_seg - 1) // B_UNROLL, b_body, 0)
        cp_aout.wait()
        cp_bout(0, 1, sem_out.at[1]).wait()
        cp_bout(n_seg - B_UNROLL, B_UNROLL, sem_out.at[2]).wait()

    qbuf = pltpu.VMEM((nt_d, A_CHUNK, LANES), F32)
    kbuf = pltpu.VMEM((nt_d, A_HALO + A_CHUNK, LANES), F32)
    obuf = pltpu.VMEM((A_CHUNK, D), F32)
    hbuf = pltpu.VMEM((L, D), F32)
    scratch = [
        pltpu.VMEM((S, D), BF16),
        pltpu.VMEM((D, 3 * D), BF16),
        pltpu.VMEM((D, D), BF16),
        pltpu.VMEM((nt_d, 3 * D // 2, LANES), U32),
        pltpu.VMEM((3 * D // 2, D), U32),
        pltpu.VMEM((nt_d, D // 2, LANES), U32),
        pltpu.VMEM((D // 2, D), U32),
        qbuf, qbuf, kbuf, kbuf, kbuf, kbuf, obuf, obuf,
        pltpu.VMEM((S, D), BF16),
        pltpu.VMEM((S, D), BF16),
        pltpu.VMEM((M, D), BF16),
        pltpu.VMEM((3, n_pair, PW, D), BF16),
        pltpu.VMEM((n_pair, PW, D), BF16),
        pltpu.VMEM((n_pair, D // 2, 3 * PW), U32),
        pltpu.VMEM((n_pair, PW // 2, D), U32),
        hbuf, hbuf, hbuf, hbuf,
        pltpu.VMEM((S, D), BF16),
        pltpu.SemaphoreType.DMA((sem_wo + n_pair,)),
        pltpu.SemaphoreType.DMA((3,)),
    ]
    return pl.pallas_call(
        kernel,
        out_shape=jax.ShapeDtypeStruct((S, 2 * D), BF16),
        in_specs=[pl.BlockSpec(memory_space=pl.ANY)] * 9,
        out_specs=pl.BlockSpec(memory_space=pl.ANY),
        scratch_shapes=scratch,
        compiler_params=pltpu.CompilerParams(vmem_limit_bytes=110 * 1024 * 1024),
    )


def pallas_concat_heads__sliding_local_dilated__memory_aug_recurrent_mem_tr__prompt_kernel(
    A_x, A_wqkv, A_wo, B_x, B_mem0, B_Wq, B_Wk, B_Wv, B_Wo, B_seg_len,
):
    batch, S, D = B_x.shape
    M = B_mem0.shape[1]
    _, H, Dh = B_Wq.shape
    assert batch == 1 and A_x.shape == B_x.shape

    def pairs(w):
        return jnp.transpose(w, (1, 2, 0)).reshape(H // 2, 2 * Dh, D)

    out = _build(S, D, M, H, Dh, int(B_seg_len))(
        A_x.reshape(S, D), A_wqkv, A_wo, B_x.reshape(S, D), B_mem0.reshape(M, D),
        pairs(B_Wq), pairs(B_Wk), pairs(B_Wv), B_Wo.reshape(H // 2, 2 * Dh, D))
    return out.reshape(1, S, 2 * D)
```

```python
import jax
import jax.numpy as jnp
from jax import lax
import jax.experimental.pallas as pl
import jax.experimental.pallas.tpu as pltpu

F32 = jnp.float32
BF16 = jnp.bfloat16
U32 = jnp.uint32

LANES = 128
A_HEADS = 32
A_WIN = 8
A_DIL = 2
A_CHUNK = 128
A_HALO = 16
B_UNROLL = 3
WO_GROUP = 4
NEG = -1000000000.0


def _nn(a, b):
    return lax.dot_general(a, b, (((1,), (0,)), ((), ())), preferred_element_type=F32)


def _nt(a, b):
    return lax.dot_general(a, b, (((1,), (1,)), ((), ())), preferred_element_type=F32)


def _build(S, D, M, H, Dh, seg):
    nt_d = D // LANES
    a_dh = D // A_HEADS
    n_chunk = S // A_CHUNK
    n_pair = H // 2
    PW = 2 * Dh
    L = M + seg
    n_seg = S // seg
    assert D % LANES == 0 and 4 * A_HEADS == LANES and a_dh == 4 * nt_d
    assert PW == 3 * LANES and n_pair == n_chunk and n_chunk % 2 == 0
    assert M % 8 == 0 and seg % 16 == 0 and 2 * L <= LANES
    assert (n_seg - 1) % B_UNROLL == 0 and n_pair % WO_GROUP == 0
    sem_aw = 4
    sem_ax = sem_aw + nt_d
    sem_w = sem_ax + n_chunk
    sem_wo = sem_w + n_pair
    a_scale = a_dh ** -0.5
    b_scale = Dh ** -0.5

    def kernel(ax_hbm, awqkv_hbm, awo_hbm, bx_hbm, mem_hbm, wq_hbm, wk_hbm, wv_hbm, wo_hbm,
               out_hbm,
               ax, awqkv_raw, awo_raw, aw_t, awp, awo_t, awop,
               q0, q1, k0, k1, v0, v1, o0, o1, a_out,
               bx, mem0, wraw, wo_raw, wqkv, wo, h0, h1, h2, h3, b_out,
               sem_in, sem_out):
        cp_awo = pltpu.make_async_copy(awo_hbm, awo_raw, sem_in.at[0])
        cp_mem = pltpu.make_async_copy(mem_hbm, mem0, sem_in.at[1])
        cp_bx0 = pltpu.make_async_copy(bx_hbm.at[pl.ds(0, seg)], bx.at[pl.ds(0, seg)], sem_in.at[2])
        cp_bx1 = pltpu.make_async_copy(bx_hbm.at[pl.ds(seg, S - seg)], bx.at[pl.ds(seg, S - seg)], sem_in.at[3])
        cp_aout = pltpu.make_async_copy(a_out, out_hbm.at[:, pl.ds(0, D)], sem_out.at[0])

        def cp_awqkv(t):
            rows = pl.ds(t * LANES, LANES)
            return pltpu.make_async_copy(awqkv_hbm.at[rows], awqkv_raw.at[rows], sem_in.at[sem_aw + t])

        def cp_ax(c):
            rows = pl.ds(pl.multiple_of(c * A_CHUNK, A_CHUNK), A_CHUNK)
            return pltpu.make_async_copy(ax_hbm.at[rows], ax.at[rows], sem_in.at[sem_ax + c])

        def cp_w(j, g):
            src = (wq_hbm, wk_hbm, wv_hbm)[j]
            return pltpu.make_async_copy(src.at[g], wraw.at[j, g], sem_in.at[sem_w + g])

        def cp_wo(i):
            grp = pl.ds(i * WO_GROUP, WO_GROUP)
            return pltpu.make_async_copy(wo_hbm.at[grp], wo_raw.at[grp], sem_in.at[sem_wo + i])

        def cp_bout(s0, n, sem):
            rows = pl.ds(pl.multiple_of(s0 * seg, seg), n * seg)
            return pltpu.make_async_copy(b_out.at[rows], out_hbm.at[rows, pl.ds(D, D)], sem)

        for t in range(nt_d):
            cp_awqkv(t).start()
        cp_ax(0).start()
        cp_ax(1).start()
        cp_awo.start()

        def start_pairs(lo, hi):
            for g in range(lo, hi):
                if g + 2 < n_chunk:
                    cp_ax(g + 2).start()
                for j in range(3):
                    cp_w(j, g).start()

        start_pairs(0, n_pair // 2)

        def reorder(src, dst, base):
            for j in range(a_dh // 2):
                for t in range(nt_d):
                    x = src[t, pl.ds(base + j, A_HEADS, stride=a_dh // 2), :]
                    even = pltpu.bitcast(x << 16, F32)
                    odd = pltpu.bitcast((x >> 16) << 16, F32)
                    y = jnp.concatenate([even, odd], axis=0).astype(BF16)
                    dst[pl.ds(base + A_HEADS * j, A_HEADS), t * LANES:(t + 1) * LANES] = pltpu.bitcast(y, U32)

        for t in range(nt_d):
            cp_awqkv(t).wait()
            aw_t[t] = pltpu.bitcast(awqkv_raw[t * LANES:(t + 1) * LANES, :].T, U32)
        for p in range(3):
            reorder(aw_t, awp, p * D // 2)

        def a_proj(c, bufs, n):
            q, k, v = bufs
            x = ax[pl.ds(pl.multiple_of(c * A_CHUNK, A_CHUNK), A_CHUNK), :]
            w = pltpu.bitcast(awp[n * (LANES // 2):(n + 1) * (LANES // 2), :], BF16)
            r = _nt(x, w)
            part, t = divmod(n, nt_d)
            if part == 0:
                q[t] = r
            else:
                (k, v)[part - 1][t, A_HALO:, :] = r

        def a_dots(bufs, r):
            q, k, _ = bufs
            qs = [q[t, 8 * r:8 * r + 8, :] for t in range(nt_d)]
            part = []
            for w in range(A_WIN):
                off = A_HALO + 8 * r - A_DIL * w
                s = qs[0] * k[0, off:off + 8, :]
                for t in range(1, nt_d):
                    s = s + qs[t] * k[t, off:off + 8, :]
                part.append(s + pltpu.roll(s, 2 * A_HEADS, 1))
            return part

        def a_fold(part):
            return [s + pltpu.roll(s, A_HEADS, 1) for s in part]

        def a_mix(c, bufs, o, r, dots):
            v = bufs[2]
            logits = []
            for w, s in enumerate(dots):
                s = s * a_scale
                if 8 * r < A_DIL * w:
                    pos = c * A_CHUNK + 8 * r + lax.broadcasted_iota(jnp.int32, (8, LANES), 0)
                    s = jnp.where(pos >= A_DIL * w, s, NEG)
                logits.append(s)
            m = logits[0]
            for s in logits[1:]:
                m = jnp.maximum(m, s)
            es = [jnp.exp(s - m) for s in logits]
            den = es[0]
            for e in es[1:]:
                den = den + e
            inv = 1.0 / den
            ps = [e * inv for e in es]
            for t in range(nt_d):
                acc = None
                for w in range(A_WIN):
                    off = A_HALO + 8 * r - A_DIL * w
                    term = ps[w] * v[t, off:off + 8, :]
                    acc = term if acc is None else acc + term
                o[8 * r:8 * r + 8, t * LANES:(t + 1) * LANES] = acc

        def a_oproj(c, o, t):
            w = pltpu.bitcast(awop[:, t * LANES:(t + 1) * LANES], BF16)
            r = _nn(o[...], w)
            a_out[pl.ds(pl.multiple_of(c * A_CHUNK, A_CHUNK), A_CHUNK), t * LANES:(t + 1) * LANES] = r.astype(BF16)

        def b_prep(g, i):
            j, t = divmod(i, PW // LANES)
            blk = wraw[j, g, t * LANES:(t + 1) * LANES, :]
            wqkv[g, :, i * LANES:(i + 1) * LANES] = pltpu.bitcast(blk.T, U32)

        n_proj = 3 * nt_d
        n_grp = A_CHUNK // 8
        n_slab = 3 * PW // LANES

        def a_step(c, cur, nxt, o_cur, o_prev, do_proj, do_oproj):
            if do_proj:
                cp_ax(c + 1).wait()
            if do_oproj:
                for j in range(3):
                    cp_w(j, c - 1).wait()
            if do_proj:
                for src, dst in ((cur[1], nxt[1]), (cur[2], nxt[2])):
                    for t in range(nt_d):
                        dst[t, 0:A_HALO, :] = src[t, A_CHUNK:A_CHUNK + A_HALO, :]
            mxu = []
            if do_oproj:
                mxu += [(lambda t=t: a_oproj(c - 1, o_prev, t)) for t in range(nt_d)]
            if do_proj:
                mxu += [(lambda n=n: a_proj(c + 1, nxt, n)) for n in range(n_proj)]
            done = 0
            st = {}
            n_slot = n_grp + 2
            for r in range(n_slot):
                upto = (r + 1) * len(mxu) // n_slot
                for f in mxu[done:upto]:
                    f()
                done = upto
                if r < n_grp:
                    st[r] = a_dots(cur, r)
                if 0 <= r - 1 < n_grp:
                    st[r - 1] = a_fold(st[r - 1])
                if do_oproj and r % 2 == 0 and r // 2 < n_slab:
                    b_prep(c - 1, r // 2)
                if 0 <= r - 2 < n_grp:
                    a_mix(c, cur, o_cur, r - 2, st.pop(r - 2))

        buf0 = (q0, k0, v0)
        buf1 = (q1, k1, v1)
        cp_ax(0).wait()
        cp_awo.wait()
        for n in range(n_proj):
            a_proj(0, buf0, n)
        for t in range(nt_d):
            awo_t[t] = pltpu.bitcast(awo_raw[:, t * LANES:(t + 1) * LANES], U32)
        reorder(awo_t, awop, 0)
        for t in range(nt_d):
            k0[t, 0:A_HALO, :] = jnp.broadcast_to(k0[t, A_HALO:A_HALO + 1, :], (A_HALO, LANES))
            v0[t, 0:A_HALO, :] = jnp.broadcast_to(v0[t, A_HALO:A_HALO + 1, :], (A_HALO, LANES))
        a_step(0, buf0, buf1, o0, o1, True, False)
        start_pairs(n_pair // 2, n_pair)
        cp_mem.start()
        cp_bx0.start()
        for i in range(n_pair // WO_GROUP):
            cp_wo(i).start()
        cp_bx1.start()

        def a_body(i, carry):
            a_step(2 * i + 1, buf1, buf0, o1, o0, True, True)
            a_step(2 * i + 2, buf0, buf1, o0, o1, True, True)
            return carry

        lax.fori_loop(0, n_chunk // 2 - 1, a_body, 0)
        a_step(n_chunk - 1, buf1, buf0, o1, o0, False, True)
        for j in range(3):
            cp_w(j, n_pair - 1).wait()
        cp_mem.wait()
        cp_bx0.wait()
        for t in range(nt_d):
            a_oproj(n_chunk - 1, o1, t)
        for i in range(n_slab):
            b_prep(n_pair - 1, i)

        def b_step(s, h_ref, h_next, first_step=False, chained=False):
            r0 = pl.multiple_of(s * seg, seg)
            h_ref[M:L, :] = bx[pl.ds(r0, seg), :].astype(F32)
            low = lax.broadcasted_iota(jnp.int32, (L, LANES), 1) < Dh - LANES
            col = lax.broadcasted_iota(jnp.int32, (L, 2 * L), 1)
            row = lax.broadcasted_iota(jnp.int32, (L, 2 * L), 0)
            first = col < L
            allow = (row < M) | (row >= jnp.where(first, col, col - L))
            zero = jnp.zeros((L, LANES), F32)

            def blockdiag(x):
                t0, t1, t2 = x[:, 0:LANES], x[:, LANES:2 * LANES], x[:, 2 * LANES:3 * LANES]
                top = jnp.concatenate([t0, jnp.where(low, t1, 0.0), zero], axis=1)
                bot = jnp.concatenate([zero, jnp.where(low, 0.0, t1), t2], axis=1)
                return jnp.concatenate([top, bot], axis=0).astype(BF16)

            st = {}
            acc = []

            def proj(g):
                if chained and g == 0:
                    r = None
                    for t in range(nt_d):
                        w = pltpu.bitcast(wqkv[g, t * (LANES // 2):(t + 1) * (LANES // 2), :], BF16)
                        part = _nn(h_ref[:, t * LANES:(t + 1) * LANES], w)
                        r = part if r is None else r + part
                else:
                    r = _nn(h_ref[...], pltpu.bitcast(wqkv[g], BF16))
                st[g] = dict(q=r[:, 0:PW], k=blockdiag(r[:, PW:2 * PW]), v=blockdiag(r[:, 2 * PW:3 * PW]))

            def scores(g):
                d = st[g]
                sc = jnp.where(allow, _nt(d['q'], d['k']) * b_scale, NEG)
                m0 = jnp.max(jnp.where(first, sc, -jnp.inf), axis=1, keepdims=True)
                m1 = jnp.max(jnp.where(first, -jnp.inf, sc), axis=1, keepdims=True)
                e = jnp.exp(sc - jnp.where(first, m0, m1))
                l0 = jnp.sum(jnp.where(first, e, 0.0), axis=1, keepdims=True)
                l1 = jnp.sum(jnp.where(first, 0.0, e), axis=1, keepdims=True)
                d['p'] = e / jnp.where(first, l0, l1)

            def mix(g):
                d = st[g]
                d['o'] = _nn(d['p'], d['v'])

            def oproj(g):
                if first_step:
                    if g % WO_GROUP == 0:
                        cp_wo(g // WO_GROUP).wait()
                    w = wo_raw[g]
                    wo[g] = pltpu.bitcast(w, U32)
                else:
                    w = pltpu.bitcast(wo[g], BF16)
                r = _nn(st.pop(g)['o'], w)
                acc[:] = [r if not acc else acc[0] + r]

            stages = ((proj, 0), (scores, 1), (mix, 4), (oproj, n_pair if first_step else 6))
            for t in range(n_pair + stages[-1][1]):
                for fn, lag in stages:
                    if 0 <= t - lag < n_pair:
                        fn(t - lag)
            for t in range(nt_d):
                cols = slice(t * LANES, (t + 1) * LANES)
                h_next[0:M, cols] = acc[0][0:M, cols].astype(BF16).astype(F32)
            b_out[pl.ds(r0, seg), :] = acc[0][M:L].astype(BF16)

        hs = (h1, h2, h3)
        h0[0:M, :] = mem0[...].astype(F32)
        b_step(0, h0, hs[0], first_step=True)
        cp_bx1.wait()
        cp_aout.start()
        cp_bout(0, 1, sem_out.at[1]).start()

        def b_body(i, carry):
            s0 = 1 + B_UNROLL * i
            for u in range(B_UNROLL):
                b_step(s0 + u, hs[u], hs[(u + 1) % B_UNROLL], chained=u > 0)

            @pl.when(i > 0)
            def _():
                cp_bout(s0 - B_UNROLL, B_UNROLL, sem_out.at[2]).wait()

            cp_bout(s0, B_UNROLL, sem_out.at[2]).start()
            return carry

        lax.fori_loop(0, (n_seg - 1) // B_UNROLL, b_body, 0)
        cp_aout.wait()
        cp_bout(0, 1, sem_out.at[1]).wait()
        cp_bout(n_seg - B_UNROLL, B_UNROLL, sem_out.at[2]).wait()

    qbuf = pltpu.VMEM((nt_d, A_CHUNK, LANES), F32)
    kbuf = pltpu.VMEM((nt_d, A_HALO + A_CHUNK, LANES), F32)
    obuf = pltpu.VMEM((A_CHUNK, D), F32)
    hbuf = pltpu.VMEM((L, D), F32)
    scratch = [
        pltpu.VMEM((S, D), BF16),
        pltpu.VMEM((D, 3 * D), BF16),
        pltpu.VMEM((D, D), BF16),
        pltpu.VMEM((nt_d, 3 * D // 2, LANES), U32),
        pltpu.VMEM((3 * D // 2, D), U32),
        pltpu.VMEM((nt_d, D // 2, LANES), U32),
        pltpu.VMEM((D // 2, D), U32),
        qbuf, qbuf, kbuf, kbuf, kbuf, kbuf, obuf, obuf,
        pltpu.VMEM((S, D), BF16),
        pltpu.VMEM((S, D), BF16),
        pltpu.VMEM((M, D), BF16),
        pltpu.VMEM((3, n_pair, PW, D), BF16),
        pltpu.VMEM((n_pair, PW, D), BF16),
        pltpu.VMEM((n_pair, D // 2, 3 * PW), U32),
        pltpu.VMEM((n_pair, PW // 2, D), U32),
        hbuf, hbuf, hbuf, hbuf,
        pltpu.VMEM((S, D), BF16),
        pltpu.SemaphoreType.DMA((sem_wo + n_pair // WO_GROUP,)),
        pltpu.SemaphoreType.DMA((3,)),
    ]
    return pl.pallas_call(
        kernel,
        out_shape=jax.ShapeDtypeStruct((S, 2 * D), BF16),
        in_specs=[pl.BlockSpec(memory_space=pl.ANY)] * 9,
        out_specs=pl.BlockSpec(memory_space=pl.ANY),
        scratch_shapes=scratch,
        compiler_params=pltpu.CompilerParams(vmem_limit_bytes=110 * 1024 * 1024),
    )


def pallas_concat_heads__sliding_local_dilated__memory_aug_recurrent_mem_tr__prompt_kernel(
    A_x, A_wqkv, A_wo, B_x, B_mem0, B_Wq, B_Wk, B_Wv, B_Wo, B_seg_len,
):
    batch, S, D = B_x.shape
    M = B_mem0.shape[1]
    _, H, Dh = B_Wq.shape
    assert batch == 1 and A_x.shape == B_x.shape

    def pairs(w):
        return jnp.transpose(w, (1, 2, 0)).reshape(H // 2, 2 * Dh, D)

    out = _build(S, D, M, H, Dh, int(B_seg_len))(
        A_x.reshape(S, D), A_wqkv, A_wo, B_x.reshape(S, D), B_mem0.reshape(M, D),
        pairs(B_Wq), pairs(B_Wk), pairs(B_Wv), B_Wo.reshape(H // 2, 2 * Dh, D))
    return out.reshape(1, S, 2 * D)
```

```python
import functools

import jax
import jax.numpy as jnp
from jax import lax
import jax.experimental.pallas as pl
import jax.experimental.pallas.tpu as pltpu

F32 = jnp.float32
BF16 = jnp.bfloat16
U32 = jnp.uint32

LANES = 128
A_HEADS = 32
A_WIN = 8
A_DIL = 2
A_CHUNK = 128
A_HALO = 16
B_UNROLL = 3
WO_GROUP = 4
NEG = -1000000000.0


def _nn(a, b):
    return lax.dot_general(a, b, (((1,), (0,)), ((), ())), preferred_element_type=F32)


def _nt(a, b):
    return lax.dot_general(a, b, (((1,), (1,)), ((), ())), preferred_element_type=F32)


def _tile(t):
    return slice(t * LANES, (t + 1) * LANES)


def _interleave(*lists):
    keyed = [((i + 0.5) / len(tasks), k, f) for k, tasks in enumerate(lists) for i, f in enumerate(tasks)]
    return [f for _, _, f in sorted(keyed, key=lambda e: e[:2])]


def _pipeline(n, stages):
    def slot(t):
        for fn, lag in stages:
            if 0 <= t - lag < n:
                fn(t - lag)
    return [functools.partial(slot, t) for t in range(n + max(lag for _, lag in stages))]


def _run(tasks):
    for f in tasks:
        f()


def _build(S, D, M, H, Dh, seg):
    nt_d = D // LANES
    a_dh = D // A_HEADS
    n_chunk = S // A_CHUNK
    n_pair = H // 2
    PW = 2 * Dh
    L = M + seg
    n_seg = S // seg
    assert D % LANES == 0 and 4 * A_HEADS == LANES and a_dh == 4 * nt_d
    assert PW == 3 * LANES and n_pair == n_chunk and n_chunk % 2 == 0
    assert M % 8 == 0 and seg % 16 == 0 and 2 * L <= LANES
    assert (n_seg - 1) % B_UNROLL == 0 and n_pair % WO_GROUP == 0
    sem_head, sem_bx0, sem_bx1, sem_aw = 0, 1, 2, 3
    sem_pair = sem_aw + 3
    sem_wo = sem_pair + n_pair
    bx_head = (1 + B_UNROLL) * seg
    a_scale = a_dh ** -0.5
    b_scale = Dh ** -0.5
    part = functools.partial

    def kernel(ax_hbm, awqkv_hbm, awo_hbm, bx_hbm, mem_hbm, wq_hbm, wk_hbm, wv_hbm, wo_hbm,
               out_hbm,
               ax, awqkv_raw, awo_raw, aw_t, awp, awo_t, awop,
               qkv0, qkv1, o0, o1, a_out,
               bx, mem0, wraw, wo_raw, wqkv, wo, h0, h1, h2, h3, b_out,
               sem_in, sem_out):
        copy = pltpu.make_async_copy

        def cp_awqkv(p):
            cols = pl.ds(p * D, D)
            return copy(awqkv_hbm.at[:, cols], awqkv_raw.at[:, cols], sem_in.at[sem_aw + p])

        def cp_ax(c, n, sem):
            rows = pl.ds(pl.multiple_of(c * A_CHUNK, A_CHUNK), n * A_CHUNK)
            return copy(ax_hbm.at[rows], ax.at[rows], sem_in.at[sem])

        def cps_pair(g, with_x):
            cps = [cp_ax(g + 2, 1, sem_pair + g)] if with_x else []
            return cps + [copy(w.at[g], wraw.at[j, g], sem_in.at[sem_pair + g])
                          for j, w in enumerate((wq_hbm, wk_hbm, wv_hbm))]

        def cp_wo(i):
            grp = pl.ds(i * WO_GROUP, WO_GROUP)
            return copy(wo_hbm.at[grp], wo_raw.at[grp], sem_in.at[sem_wo + i])

        def cp_bout(s0, n, sem):
            rows = pl.ds(pl.multiple_of(s0 * seg, seg), n * seg)
            return copy(b_out.at[rows], out_hbm.at[rows, pl.ds(D, D)], sem_out.at[sem])

        cp_ax0 = cp_ax(0, 2, sem_aw)
        cp_awo = copy(awo_hbm, awo_raw, sem_in.at[sem_head])
        cps_b0 = [copy(mem_hbm, mem0, sem_in.at[sem_bx0]),
                  copy(bx_hbm.at[pl.ds(0, bx_head)], bx.at[pl.ds(0, bx_head)], sem_in.at[sem_bx0])]
        cp_bx1 = copy(bx_hbm.at[pl.ds(bx_head, S - bx_head)], bx.at[pl.ds(bx_head, S - bx_head)],
                      sem_in.at[sem_bx1])
        cp_aout = copy(a_out, out_hbm.at[:, pl.ds(0, D)], sem_out.at[0])
        n_iter = n_chunk // 2 - 1

        early = [cp_awqkv(0), cp_ax0, cp_awqkv(1), cp_awqkv(2), cp_awo]
        late = []
        for g in range(n_pair):
            (early if g < n_pair // 2 else late).extend(cps_pair(g, g + 2 < n_chunk))
        late += cps_b0 + [cp_wo(i) for i in range(n_pair // WO_GROUP)] + [cp_bx1]
        for cp in early:
            cp.start()

        def reorder(src, dst, base, j):
            for t in range(nt_d):
                x = src[t, pl.ds(base + j, A_HEADS, stride=a_dh // 2), :]
                even = pltpu.bitcast(x << 16, F32)
                odd = pltpu.bitcast((x >> 16) << 16, F32)
                y = jnp.concatenate([even, odd], axis=0).astype(BF16)
                dst[pl.ds(base + A_HEADS * j, A_HEADS), _tile(t)] = pltpu.bitcast(y, U32)

        def a_proj(c, buf, n):
            x = ax[pl.ds(pl.multiple_of(c * A_CHUNK, A_CHUNK), A_CHUNK), :]
            w = pltpu.bitcast(awp[n * (LANES // 2):(n + 1) * (LANES // 2), :], BF16)
            r = _nt(x, w)
            buf[n, A_HALO:, :] = r

        def a_halo(cur, nxt):
            for n in range(nt_d, 3 * nt_d):
                nxt[n, 0:A_HALO, :] = cur[n, A_CHUNK:A_CHUNK + A_HALO, :]

        def a_attn(c, buf, o):
            st = {}

            def dots(r):
                qs = [buf[t, A_HALO + 8 * r:A_HALO + 8 * r + 8, :] for t in range(nt_d)]
                st[r] = []
                for w in range(A_WIN):
                    off = A_HALO + 8 * r - A_DIL * w
                    s = qs[0] * buf[nt_d, off:off + 8, :]
                    for t in range(1, nt_d):
                        s = s + qs[t] * buf[nt_d + t, off:off + 8, :]
                    st[r].append(s + pltpu.roll(s, 2 * A_HEADS, 1))

            def fold(r):
                st[r] = [s + pltpu.roll(s, A_HEADS, 1) for s in st[r]]

            def mix(r):
                logits = []
                for w, s in enumerate(st.pop(r)):
                    s = s * a_scale
                    if 8 * r < A_DIL * w:
                        pos = c * A_CHUNK + 8 * r + lax.broadcasted_iota(jnp.int32, (8, LANES), 0)
                        s = jnp.where(pos >= A_DIL * w, s, NEG)
                    logits.append(s)
                m = functools.reduce(jnp.maximum, logits)
                es = [jnp.exp(s - m) for s in logits]
                inv = 1.0 / functools.reduce(jnp.add, es)
                ps = [e * inv for e in es]
                for t in range(nt_d):
                    acc = None
                    for w in range(A_WIN):
                        off = A_HALO + 8 * r - A_DIL * w
                        term = ps[w] * buf[2 * nt_d + t, off:off + 8, :]
                        acc = term if acc is None else acc + term
                    o[8 * r:8 * r + 8, _tile(t)] = acc

            return _pipeline(A_CHUNK // 8, ((dots, 0), (fold, 1), (mix, 2)))

        def a_oproj(c, o, t):
            r = _nn(o[...], pltpu.bitcast(awop[:, _tile(t)], BF16))
            a_out[pl.ds(pl.multiple_of(c * A_CHUNK, A_CHUNK), A_CHUNK), _tile(t)] = r.astype(BF16)

        def b_prep(g):
            def slab(i):
                j, t = divmod(i, PW // LANES)
                wqkv[g, :, _tile(i)] = pltpu.bitcast(wraw[j, g, _tile(t), :].T, U32)
            return [part(slab, i) for i in range(3 * PW // LANES)]

        def proj_tasks(c, bufs):
            return [part(a_proj, c, bufs, n) for n in range(3 * nt_d)]

        def oproj_tasks(c, o):
            return [part(a_oproj, c, o, t) for t in range(nt_d)]

        buf0, buf1 = qkv0, qkv1
        for p in range(3):
            cp_awqkv(p).wait()
            if p == 0:
                cp_ax0.wait()
            for t in range(nt_d):
                aw_t[t, pl.ds(p * D // 2, D // 2), :] = pltpu.bitcast(
                    awqkv_raw[_tile(t), p * D:(p + 1) * D].T, U32)
            for t in range(nt_d):
                reorder(aw_t, awp, p * D // 2, 2 * t)
                reorder(aw_t, awp, p * D // 2, 2 * t + 1)
                a_proj(0, buf0, p * nt_d + t)
        cp_awo.wait()
        for t in range(nt_d):
            for n in (nt_d + t, 2 * nt_d + t):
                buf0[n, 0:A_HALO, :] = jnp.broadcast_to(buf0[n, A_HALO:A_HALO + 1, :], (A_HALO, LANES))
            awo_t[t] = pltpu.bitcast(awo_raw[:, _tile(t)], U32)
        a_halo(buf0, buf1)
        _run(_interleave(proj_tasks(1, buf1), a_attn(0, buf0, o0),
                         [part(reorder, awo_t, awop, 0, j) for j in range(a_dh // 2)]))
        for cp in late:
            cp.start()

        def a_body(i, carry):
            for c, cur, nxt, o_cur, o_prev in ((2 * i + 1, buf1, buf0, o1, o0), (2 * i + 2, buf0, buf1, o0, o1)):
                for cp in cps_pair(c - 1, True):
                    cp.wait()
                a_halo(cur, nxt)
                _run(_interleave(oproj_tasks(c - 1, o_prev) + proj_tasks(c + 1, nxt),
                                 a_attn(c, cur, o_cur) + b_prep(c - 1)))
            return carry

        lax.fori_loop(0, n_iter, a_body, 0)

        def b_step(s, h_ref, h_next, first_step=False, chained=False):
            r0 = pl.multiple_of(s * seg, seg)
            h_ref[M:L, :] = bx[pl.ds(r0, seg), :].astype(F32)
            low = lax.broadcasted_iota(jnp.int32, (L, LANES), 1) < Dh - LANES
            col = lax.broadcasted_iota(jnp.int32, (L, 2 * L), 1)
            row = lax.broadcasted_iota(jnp.int32, (L, 2 * L), 0)
            first = col < L
            allow = (row < M) | (row >= jnp.where(first, col, col - L))
            zero = jnp.zeros((L, LANES), F32)

            def blockdiag(x):
                t0, t1, t2 = x[:, _tile(0)], x[:, _tile(1)], x[:, _tile(2)]
                top = jnp.concatenate([t0, jnp.where(low, t1, 0.0), zero], axis=1)
                bot = jnp.concatenate([zero, jnp.where(low, 0.0, t1), t2], axis=1)
                return jnp.concatenate([top, bot], axis=0).astype(BF16)

            st = {}

            def proj(g):
                if chained and g == 0:
                    r = None
                    for t in range(nt_d):
                        w = pltpu.bitcast(wqkv[g, t * (LANES // 2):(t + 1) * (LANES // 2), :], BF16)
                        term = _nn(h_ref[:, _tile(t)], w)
                        r = term if r is None else r + term
                else:
                    r = _nn(h_ref[...], pltpu.bitcast(wqkv[g], BF16))
                st[g] = dict(q=r[:, 0:PW], k=blockdiag(r[:, PW:2 * PW]), v=blockdiag(r[:, 2 * PW:3 * PW]))

            def scores(g):
                d = st[g]
                sc = jnp.where(allow, _nt(d['q'], d['k']) * b_scale, NEG)
                m0 = jnp.max(jnp.where(first, sc, -jnp.inf), axis=1, keepdims=True)
                m1 = jnp.max(jnp.where(first, -jnp.inf, sc), axis=1, keepdims=True)
                e = jnp.exp(sc - jnp.where(first, m0, m1))
                l0 = jnp.sum(jnp.where(first, e, 0.0), axis=1, keepdims=True)
                l1 = jnp.sum(jnp.where(first, 0.0, e), axis=1, keepdims=True)
                d['p'] = e / jnp.where(first, l0, l1)

            def mix(g):
                d = st[g]
                d['o'] = _nn(d['p'], d['v'])

            def oproj(g):
                if first_step:
                    if g % WO_GROUP == 0:
                        cp_wo(g // WO_GROUP).wait()
                    w = wo_raw[g]
                    wo[g] = pltpu.bitcast(w, U32)
                else:
                    w = pltpu.bitcast(wo[g], BF16)
                r = _nn(st.pop(g)['o'], w)
                st['acc'] = st['acc'] + r if g else r

            def finish():
                out = st.pop('acc')
                for t in range(nt_d):
                    h_next[0:M, _tile(t)] = out[0:M, _tile(t)].astype(BF16).astype(F32)
                b_out[pl.ds(r0, seg), :] = out[M:L].astype(BF16)

            stages = ((proj, 0), (scores, 1), (mix, 4), (oproj, n_pair if first_step else 6))
            return _pipeline(n_pair, stages) + [finish]

        hs = (h1, h2, h3)
        for cp in cps_pair(n_pair - 2, False) + cps_pair(n_pair - 1, False) + cps_b0:
            cp.wait()
        h0[0:M, :] = mem0[...].astype(F32)
        first_seg = b_step(0, h0, hs[0], first_step=True)
        _run(_interleave(oproj_tasks(n_chunk - 2, o0) + first_seg[:4], a_attn(n_chunk - 1, buf1, o1)))
        _run(_interleave(oproj_tasks(n_chunk - 1, o1) + first_seg[4:8], b_prep(n_pair - 2) + b_prep(n_pair - 1)))
        _run(first_seg[8:])
        cp_aout.start()
        cp_bout(0, 1, 1).start()

        def b_body(i, carry):
            s0 = 1 + B_UNROLL * i
            for u in range(B_UNROLL):
                _run(b_step(s0 + u, hs[u], hs[(u + 1) % B_UNROLL], chained=u > 0))

            @pl.when(i == 0)
            def _():
                cp_bx1.wait()

            @pl.when(i > 0)
            def _():
                cp_bout(s0 - B_UNROLL, B_UNROLL, 2).wait()

            cp_bout(s0, B_UNROLL, 2).start()
            return carry

        lax.fori_loop(0, (n_seg - 1) // B_UNROLL, b_body, 0)
        cp_aout.wait()
        cp_bout(0, 1, 1).wait()
        cp_bout(n_seg - B_UNROLL, B_UNROLL, 2).wait()

    qkvbuf = pltpu.VMEM((3 * nt_d, A_HALO + A_CHUNK, LANES), F32)
    obuf = pltpu.VMEM((A_CHUNK, D), F32)
    hbuf = pltpu.VMEM((L, D), F32)
    scratch = [
        pltpu.VMEM((S, D), BF16),
        pltpu.VMEM((D, 3 * D), BF16),
        pltpu.VMEM((D, D), BF16),
        pltpu.VMEM((nt_d, 3 * D // 2, LANES), U32),
        pltpu.VMEM((3 * D // 2, D), U32),
        pltpu.VMEM((nt_d, D // 2, LANES), U32),
        pltpu.VMEM((D // 2, D), U32),
        qkvbuf, qkvbuf, obuf, obuf,
        pltpu.VMEM((S, D), BF16),
        pltpu.VMEM((S, D), BF16),
        pltpu.VMEM((M, D), BF16),
        pltpu.VMEM((3, n_pair, PW, D), BF16),
        pltpu.VMEM((n_pair, PW, D), BF16),
        pltpu.VMEM((n_pair, D // 2, 3 * PW), U32),
        pltpu.VMEM((n_pair, PW // 2, D), U32),
        hbuf, hbuf, hbuf, hbuf,
        pltpu.VMEM((S, D), BF16),
        pltpu.SemaphoreType.DMA((sem_wo + n_pair // WO_GROUP,)),
        pltpu.SemaphoreType.DMA((3,)),
    ]
    return pl.pallas_call(
        kernel,
        out_shape=jax.ShapeDtypeStruct((S, 2 * D), BF16),
        in_specs=[pl.BlockSpec(memory_space=pl.ANY)] * 9,
        out_specs=pl.BlockSpec(memory_space=pl.ANY),
        scratch_shapes=scratch,
        compiler_params=pltpu.CompilerParams(vmem_limit_bytes=110 * 1024 * 1024),
    )


def pallas_concat_heads__sliding_local_dilated__memory_aug_recurrent_mem_tr__prompt_kernel(
    A_x, A_wqkv, A_wo, B_x, B_mem0, B_Wq, B_Wk, B_Wv, B_Wo, B_seg_len,
):
    batch, S, D = B_x.shape
    M = B_mem0.shape[1]
    _, H, Dh = B_Wq.shape
    assert batch == 1 and A_x.shape == B_x.shape

    def pairs(w):
        return jnp.transpose(w, (1, 2, 0)).reshape(H // 2, 2 * Dh, D)

    out = _build(S, D, M, H, Dh, int(B_seg_len))(
        A_x.reshape(S, D), A_wqkv, A_wo, B_x.reshape(S, D), B_mem0.reshape(M, D),
        pairs(B_Wq), pairs(B_Wk), pairs(B_Wv), B_Wo.reshape(H // 2, 2 * Dh, D))
    return out.reshape(1, S, 2 * D)
```

```python
import functools

import jax
import jax.numpy as jnp
from jax import lax
import jax.experimental.pallas as pl
import jax.experimental.pallas.tpu as pltpu

F32 = jnp.float32
BF16 = jnp.bfloat16
U32 = jnp.uint32

LANES = 128
A_HEADS = 32
A_WIN = 8
A_DIL = 2
A_CHUNK = 128
A_HALO = 16
B_UNROLL = 4
B_EARLY = 8
EARLY_Q = (1, 2)
WO_GROUP = 4
NEG = -1000000000.0


def _nn(a, b):
    return lax.dot_general(a, b, (((1,), (0,)), ((), ())), preferred_element_type=F32)


def _nt(a, b):
    return lax.dot_general(a, b, (((1,), (1,)), ((), ())), preferred_element_type=F32)


def _tile(t):
    return slice(t * LANES, (t + 1) * LANES)


def _interleave(*lists):
    keyed = [((i + 0.5) / len(tasks), k, f) for k, tasks in enumerate(lists) for i, f in enumerate(tasks)]
    return [f for _, _, f in sorted(keyed, key=lambda e: e[:2])]


def _pipeline(n, stages):
    def slot(t):
        for fn, lag in stages:
            if 0 <= t - lag < n:
                fn(t - lag)
    return [functools.partial(slot, t) for t in range(n + max(lag for _, lag in stages))]


def _run(tasks):
    for f in tasks:
        f()


def _build(S, D, M, H, Dh, seg):
    nt_d = D // LANES
    a_dh = D // A_HEADS
    n_chunk = S // A_CHUNK
    n_pair = H // 2
    PW = 2 * Dh
    L = M + seg
    n_seg = S // seg
    assert D % LANES == 0 and 4 * A_HEADS == LANES and a_dh == 4 * nt_d
    assert PW == 3 * LANES and n_pair == n_chunk and n_chunk % 2 == 0
    assert M % 8 == 0 and seg % 16 == 0 and 2 * L <= LANES
    assert n_seg % B_UNROLL == 0 and B_UNROLL % 2 == 0 and n_pair % WO_GROUP == 0
    n_group = n_pair // WO_GROUP
    sem_head, sem_bx0, sem_bx1, sem_bx2, sem_aw = range(5)
    sem_pair = sem_aw + 3
    sem_wo = sem_pair + n_pair
    a_scale = a_dh ** -0.5
    b_scale = Dh ** -0.5
    part = functools.partial

    def kernel(ax_hbm, awqkv_hbm, awo_hbm, bx_hbm, mem_hbm, wq_hbm, wk_hbm, wv_hbm, wo_hbm,
               out_hbm,
               ax, awqkv_raw, awo_raw, aw_t, awp, awo_t, awop,
               qkv0, qkv1, o0, o1, a_out,
               bx, bxe, xe, early_q, mem0, wraw, wo_raw, wqkv, wo, h0, h1, b_out,
               sem_in, sem_out):
        copy = pltpu.make_async_copy

        def cp_awqkv(p):
            cols = pl.ds(p * D, D)
            return copy(awqkv_hbm.at[:, cols], awqkv_raw.at[:, cols], sem_in.at[sem_aw + p])

        def cp_ax(c, n, sem):
            rows = pl.ds(pl.multiple_of(c * A_CHUNK, A_CHUNK), n * A_CHUNK)
            return copy(ax_hbm.at[rows], ax.at[rows], sem_in.at[sem])

        def cps_pair(g, with_x):
            cps = [cp_ax(g + 2, 1, sem_pair + g)] if with_x else []
            return cps + [copy(w.at[g], wraw.at[j, g], sem_in.at[sem_pair + g])
                          for j, w in enumerate((wq_hbm, wk_hbm, wv_hbm))]

        def cp_wo(i):
            grp = pl.ds(pl.multiple_of(i * WO_GROUP, WO_GROUP), WO_GROUP)
            return copy(wo_hbm.at[grp], wo_raw.at[grp], sem_in.at[sem_wo + i])

        def cp_bout(i):
            rows = pl.ds(pl.multiple_of(i * B_UNROLL * seg, B_UNROLL * seg), B_UNROLL * seg)
            return copy(b_out.at[rows], out_hbm.at[rows, pl.ds(D, D)], sem_out.at[1])

        cp_ax0 = cp_ax(0, 2, sem_aw)
        cp_awo = copy(awo_hbm, awo_raw, sem_in.at[sem_head])
        cps_b0 = [copy(mem_hbm, mem0, sem_in.at[sem_bx0]),
                  copy(bx_hbm.at[:, pl.ds(seg - B_EARLY, B_EARLY), :], bxe, sem_in.at[sem_bx0])]
        cp_bx_head, cp_bx_rest = (
            copy(bx_hbm.at[segs], bx.at[segs], sem_in.at[sem])
            for segs, sem in ((pl.ds(0, B_UNROLL), sem_bx1), (pl.ds(B_UNROLL, n_seg - B_UNROLL), sem_bx2)))
        cp_aout = copy(a_out, out_hbm.at[:, pl.ds(0, D)], sem_out.at[0])
        n_iter = n_chunk // 2 - 1

        early = [cp_awqkv(0), cp_ax0, cp_awqkv(1), cp_awqkv(2), cp_awo]
        late = []
        for g in range(n_chunk - 2):
            (early if g < n_pair // 2 else late).extend(cps_pair(g, True))
        late += cps_b0
        for i in range(n_group):
            late.append(cp_wo(i))
            if n_pair - n_group + i >= n_chunk - 2:
                late += cps_pair(n_pair - n_group + i, False)
        late += [cp_bx_head, cp_bx_rest]
        for cp in early:
            cp.start()

        def reorder(src, dst, base, j):
            for t in range(nt_d):
                x = src[t, pl.ds(base + j, A_HEADS, stride=a_dh // 2), :]
                even = pltpu.bitcast(x << 16, F32)
                odd = pltpu.bitcast((x >> 16) << 16, F32)
                y = jnp.concatenate([even, odd], axis=0).astype(BF16)
                dst[pl.ds(base + A_HEADS * j, A_HEADS), _tile(t)] = pltpu.bitcast(y, U32)

        def a_proj(c, buf, n):
            x = ax[pl.ds(pl.multiple_of(c * A_CHUNK, A_CHUNK), A_CHUNK), :]
            w = pltpu.bitcast(awp[n * (LANES // 2):(n + 1) * (LANES // 2), :], BF16)
            r = _nt(x, w)
            buf[n, A_HALO:, :] = r

        def a_halo(cur, nxt):
            for n in range(nt_d, 3 * nt_d):
                nxt[n, 0:A_HALO, :] = cur[n, A_CHUNK:A_CHUNK + A_HALO, :]

        def a_attn(c, buf, o):
            st = {}

            def dots(r):
                qs = [buf[t, A_HALO + 8 * r:A_HALO + 8 * r + 8, :] for t in range(nt_d)]
                st[r] = []
                for w in range(A_WIN):
                    off = A_HALO + 8 * r - A_DIL * w
                    s = qs[0] * buf[nt_d, off:off + 8, :]
                    for t in range(1, nt_d):
                        s = s + qs[t] * buf[nt_d + t, off:off + 8, :]
                    st[r].append(s + pltpu.roll(s, 2 * A_HEADS, 1))

            def fold(r):
                st[r] = [s + pltpu.roll(s, A_HEADS, 1) for s in st[r]]

            def mix(r):
                logits = []
                for w, s in enumerate(st.pop(r)):
                    s = s * a_scale
                    if 8 * r < A_DIL * w:
                        pos = c * A_CHUNK + 8 * r + lax.broadcasted_iota(jnp.int32, (8, LANES), 0)
                        s = jnp.where(pos >= A_DIL * w, s, NEG)
                    logits.append(s)
                m = functools.reduce(jnp.maximum, logits)
                es = [jnp.exp(s - m) for s in logits]
                inv = 1.0 / functools.reduce(jnp.add, es)
                ps = [e * inv for e in es]
                for t in range(nt_d):
                    acc = None
                    for w in range(A_WIN):
                        off = A_HALO + 8 * r - A_DIL * w
                        term = ps[w] * buf[2 * nt_d + t, off:off + 8, :]
                        acc = term if acc is None else acc + term
                    o[8 * r:8 * r + 8, _tile(t)] = acc

            return _pipeline(A_CHUNK // 8, ((fold, 1), (dots, 0), (mix, 2)))

        def a_oproj(c, o, t):
            r = _nn(o[...], pltpu.bitcast(awop[:, _tile(t)], BF16))
            a_out[pl.ds(pl.multiple_of(c * A_CHUNK, A_CHUNK), A_CHUNK), _tile(t)] = r.astype(BF16)

        def b_prep(g):
            def slab(i):
                j, t = divmod(i, PW // LANES)
                wqkv[g, :, _tile(i)] = pltpu.bitcast(wraw[j, g, _tile(t), :].T, U32)
            return [part(slab, i) for i in range(3 * PW // LANES)]

        def proj_tasks(c, bufs):
            return [part(a_proj, c, bufs, n) for n in range(3 * nt_d)]

        def oproj_tasks(c, o):
            return [part(a_oproj, c, o, t) for t in range(nt_d)]

        buf0, buf1 = qkv0, qkv1
        nxt_proj = proj_tasks(1, buf1)
        for p in range(3):
            cp_awqkv(p).wait()
            if p == 0:
                cp_ax0.wait()
            else:
                _run(nxt_proj[(p - 1) * nt_d:p * nt_d])
            for t in range(nt_d):
                aw_t[t, pl.ds(p * D // 2, D // 2), :] = pltpu.bitcast(
                    awqkv_raw[_tile(t), p * D:(p + 1) * D].T, U32)
            for t in range(nt_d):
                reorder(aw_t, awp, p * D // 2, 2 * t)
                reorder(aw_t, awp, p * D // 2, 2 * t + 1)
                a_proj(0, buf0, p * nt_d + t)
        cp_awo.wait()
        for t in range(nt_d):
            for n in (nt_d + t, 2 * nt_d + t):
                buf0[n, 0:A_HALO, :] = jnp.broadcast_to(buf0[n, A_HALO:A_HALO + 1, :], (A_HALO, LANES))
            awo_t[t] = pltpu.bitcast(awo_raw[:, _tile(t)], U32)
        a_halo(buf0, buf1)
        _run(_interleave(nxt_proj[2 * nt_d:], a_attn(0, buf0, o0),
                         [part(reorder, awo_t, awop, 0, j) for j in range(a_dh // 2)]))
        for cp in late:
            cp.start()

        def a_body(i, carry):
            for c, cur, nxt, o_cur, o_prev in ((2 * i + 1, buf1, buf0, o1, o0), (2 * i + 2, buf0, buf1, o0, o1)):
                for cp in cps_pair(c - 1, True):
                    cp.wait()
                a_halo(cur, nxt)
                _run(_interleave(oproj_tasks(c - 1, o_prev) + proj_tasks(c + 1, nxt),
                                 a_attn(c, cur, o_cur) + b_prep(c - 1)))
            return carry

        lax.fori_loop(0, n_iter, a_body, 0)

        def b_step(s, h_ref, h_next, chained):
            r0 = pl.multiple_of(s * seg, seg)
            h_ref[M:L, :] = bx[s].astype(F32)
            low = lax.broadcasted_iota(jnp.int32, (L, LANES), 1) < Dh - LANES
            col = lax.broadcasted_iota(jnp.int32, (L, 2 * L), 1)
            row = lax.broadcasted_iota(jnp.int32, (L, 2 * L), 0)
            first = col < L
            allow = (row < M) | (row >= jnp.where(first, col, col - L))
            zero = jnp.zeros((L, LANES), F32)

            def blockdiag(x):
                t0, t1, t2 = x[:, _tile(0)], x[:, _tile(1)], x[:, _tile(2)]
                top = jnp.concatenate([t0, jnp.where(low, t1, 0.0), zero], axis=1)
                bot = jnp.concatenate([zero, jnp.where(low, 0.0, t1), t2], axis=1)
                return jnp.concatenate([top, bot], axis=0).astype(BF16)

            st = {}

            def proj(g):
                if chained and g == 0:
                    r = None
                    for t in range(nt_d):
                        w = pltpu.bitcast(wqkv[g, t * (LANES // 2):(t + 1) * (LANES // 2), :], BF16)
                        term = _nn(h_ref[:, _tile(t)], w)
                        r = term if r is None else r + term
                elif g // n_group in EARLY_Q:
                    kv = _nn(h_ref[...], pltpu.bitcast(wqkv[g, :, PW:3 * PW], BF16))
                    q = _nn(h_ref[0:L - B_EARLY, :], pltpu.bitcast(wqkv[g, :, 0:PW], BF16))
                    rows = pl.ds(pl.multiple_of(s * B_EARLY, B_EARLY), B_EARLY)
                    q = jnp.concatenate([q, early_q[g - EARLY_Q[0] * n_group, rows, :]], axis=0)
                    r = jnp.concatenate([q, kv], axis=1)
                else:
                    r = _nn(h_ref[...], pltpu.bitcast(wqkv[g], BF16))
                st[g] = dict(q=r[:, 0:PW], k=blockdiag(r[:, PW:2 * PW]), v=blockdiag(r[:, 2 * PW:3 * PW]))

            def scores(g):
                d = st[g]
                sc = jnp.where(allow, _nt(d['q'], d['k']) * b_scale, NEG)
                m0 = jnp.max(jnp.where(first, sc, -jnp.inf), axis=1, keepdims=True)
                m1 = jnp.max(jnp.where(first, -jnp.inf, sc), axis=1, keepdims=True)
                e = jnp.exp(sc - jnp.where(first, m0, m1))
                l0 = jnp.sum(jnp.where(first, e, 0.0), axis=1, keepdims=True)
                l1 = jnp.sum(jnp.where(first, 0.0, e), axis=1, keepdims=True)
                d['p'] = e / jnp.where(first, l0, l1)

            def mix(g):
                d = st[g]
                d['o'] = _nn(d['p'], d['v'])

            def oproj(g):
                r = _nn(st.pop(g)['o'], pltpu.bitcast(wo[g], BF16))
                st['acc'] = st['acc'] + r if g else r

            def finish():
                out = st.pop('acc')
                for t in range(nt_d):
                    h_next[0:M, _tile(t)] = out[0:M, _tile(t)].astype(BF16).astype(F32)
                b_out[pl.ds(r0, seg), :] = out[M:L].astype(BF16)

            stages = ((proj, 0), (scores, 1), (mix, 4), (oproj, 6))
            return _pipeline(n_pair, stages) + [finish]

        for cp in cps_b0:
            cp.wait()
        h0[0:M, :] = mem0[...].astype(F32)
        for s in range(0, n_seg, 2):
            x = jnp.concatenate([bxe[s].astype(F32), bxe[s + 1].astype(F32)], axis=0)
            xe[s * B_EARLY // 2:(s + 2) * B_EARLY // 2, :] = pltpu.bitcast(x.astype(BF16), U32)
        _run(_interleave(oproj_tasks(n_chunk - 2, o0), a_attn(n_chunk - 1, buf1, o1)))
        _run(oproj_tasks(n_chunk - 1, o1))

        def early_body(i, carry):
            cp_wo(i).wait()

            @pl.when(n_pair - n_group + i >= n_chunk - 2)
            def _():
                for cp in cps_pair(n_pair - n_group + i, False):
                    cp.wait()

            def project(e, n):
                early_q[(e - EARLY_Q[0]) * n_group + i, :, _tile(n)] = _nn(
                    pltpu.bitcast(xe[...], BF16), pltpu.bitcast(wqkv[e * n_group + i, :, _tile(n)], BF16))

            def retile(j):
                wo[i * WO_GROUP + j] = pltpu.bitcast(wo_raw[i * WO_GROUP + j], U32)

            _run(_interleave([part(project, e, n) for e in EARLY_Q for n in range(PW // LANES)],
                             [part(retile, j) for j in range(WO_GROUP)],
                             b_prep(n_pair - n_group + i)))
            return carry

        lax.fori_loop(0, n_group, early_body, 0)
        cp_bx_head.wait()
        cp_aout.start()

        def b_body(i, carry):
            for u in range(B_UNROLL):
                _run(b_step(B_UNROLL * i + u, (h0, h1)[u % 2], (h1, h0)[u % 2], chained=u > 0))

            @pl.when(i == 0)
            def _():
                cp_bx_rest.wait()

            @pl.when(i > 0)
            def _():
                cp_bout(i - 1).wait()

            cp_bout(i).start()
            return carry

        lax.fori_loop(0, n_seg // B_UNROLL, b_body, 0)
        cp_aout.wait()
        cp_bout(n_seg // B_UNROLL - 1).wait()

    qkvbuf = pltpu.VMEM((3 * nt_d, A_HALO + A_CHUNK, LANES), F32)
    obuf = pltpu.VMEM((A_CHUNK, D), F32)
    hbuf = pltpu.VMEM((L, D), F32)
    scratch = [
        pltpu.VMEM((S, D), BF16),
        pltpu.VMEM((D, 3 * D), BF16),
        pltpu.VMEM((D, D), BF16),
        pltpu.VMEM((nt_d, 3 * D // 2, LANES), U32),
        pltpu.VMEM((3 * D // 2, D), U32),
        pltpu.VMEM((nt_d, D // 2, LANES), U32),
        pltpu.VMEM((D // 2, D), U32),
        qkvbuf, qkvbuf, obuf, obuf,
        pltpu.VMEM((S, D), BF16),
        pltpu.VMEM((n_seg, seg, D), BF16),
        pltpu.VMEM((n_seg, B_EARLY, D), BF16),
        pltpu.VMEM((n_seg * B_EARLY // 2, D), U32),
        pltpu.VMEM((n_group * len(EARLY_Q), n_seg * B_EARLY, PW), F32),
        pltpu.VMEM((M, D), BF16),
        pltpu.VMEM((3, n_pair, PW, D), BF16),
        pltpu.VMEM((n_pair, PW, D), BF16),
        pltpu.VMEM((n_pair, D // 2, 3 * PW), U32),
        pltpu.VMEM((n_pair, PW // 2, D), U32),
        hbuf, hbuf,
        pltpu.VMEM((S, D), BF16),
        pltpu.SemaphoreType.DMA((sem_wo + n_group,)),
        pltpu.SemaphoreType.DMA((2,)),
    ]
    return pl.pallas_call(
        kernel,
        out_shape=jax.ShapeDtypeStruct((S, 2 * D), BF16),
        in_specs=[pl.BlockSpec(memory_space=pl.ANY)] * 9,
        out_specs=pl.BlockSpec(memory_space=pl.ANY),
        scratch_shapes=scratch,
        compiler_params=pltpu.CompilerParams(vmem_limit_bytes=110 * 1024 * 1024),
    )


def pallas_concat_heads__sliding_local_dilated__memory_aug_recurrent_mem_tr__prompt_kernel(
    A_x, A_wqkv, A_wo, B_x, B_mem0, B_Wq, B_Wk, B_Wv, B_Wo, B_seg_len,
):
    batch, S, D = B_x.shape
    M = B_mem0.shape[1]
    _, H, Dh = B_Wq.shape
    assert batch == 1 and A_x.shape == B_x.shape

    def pairs(w):
        return jnp.transpose(w, (1, 2, 0)).reshape(H // 2, 2 * Dh, D)

    seg = int(B_seg_len)
    out = _build(S, D, M, H, Dh, seg)(
        A_x.reshape(S, D), A_wqkv, A_wo, B_x.reshape(S // seg, seg, D), B_mem0.reshape(M, D),
        pairs(B_Wq), pairs(B_Wk), pairs(B_Wv), B_Wo.reshape(H // 2, 2 * Dh, D))
    return out.reshape(1, S, 2 * D)
```

```python
import functools

import jax
import jax.numpy as jnp
from jax import lax
import jax.experimental.pallas as pl
import jax.experimental.pallas.tpu as pltpu

F32 = jnp.float32
BF16 = jnp.bfloat16
U32 = jnp.uint32

LANES = 128
A_HEADS = 32
A_WIN = 8
A_DIL = 2
A_CHUNK = 128
A_HALO = 16
B_UNROLL = 4
B_EARLY = 8
B_EARLY_SETS = 3
WO_GROUP = 4
NEG = -1000000000.0


def _nn(a, b):
    return lax.dot_general(a, b, (((1,), (0,)), ((), ())), preferred_element_type=F32)


def _nt(a, b):
    return lax.dot_general(a, b, (((1,), (1,)), ((), ())), preferred_element_type=F32)


def _tile(t):
    return slice(t * LANES, (t + 1) * LANES)


def _interleave(*lists):
    keyed = [((i + 0.5) / len(tasks), k, f) for k, tasks in enumerate(lists) for i, f in enumerate(tasks)]
    return [f for _, _, f in sorted(keyed, key=lambda e: e[:2])]


def _pipeline(n, stages):
    def slot(t):
        for fn, lag in stages:
            if 0 <= t - lag < n:
                fn(t - lag)
    return [functools.partial(slot, t) for t in range(n + max(lag for _, lag in stages))]


def _run(tasks):
    for f in tasks:
        f()


def _build(S, D, M, H, Dh, seg):
    nt_d = D // LANES
    a_dh = D // A_HEADS
    n_chunk = S // A_CHUNK
    n_pair = H // 2
    PW = 2 * Dh
    L = M + seg
    n_seg = S // seg
    assert D % LANES == 0 and 4 * A_HEADS == LANES and a_dh == 4 * nt_d
    assert PW == 3 * LANES and n_pair == n_chunk and n_chunk % 2 == 0
    assert M % 8 == 0 and seg % 16 == 0 and 2 * L <= LANES
    assert n_seg % B_UNROLL == 0 and B_UNROLL % 2 == 0 and n_pair % WO_GROUP == 0
    n_group = n_pair // WO_GROUP
    assert (B_EARLY_SETS + 1) * n_group <= n_pair
    sem_ax, sem_awo, sem_bx0, sem_bx1, sem_bx2, sem_aw = range(6)
    sem_pair = sem_aw + 3
    sem_wo = sem_pair + n_pair
    a_scale = a_dh ** -0.5
    b_scale = Dh ** -0.5
    part = functools.partial

    def kernel(ax_hbm, awqkv_hbm, awo_hbm, bx_hbm, mem_hbm, wq_hbm, wk_hbm, wv_hbm, wo_hbm,
               out_hbm,
               ax, awqkv_raw, awo_raw, aw_t, awp, awo_t, awop,
               qkv0, qkv1, o0, o1, a_out,
               bx, bxe, xe, early_q, mem0, wraw, wo_raw, wqkv, wo, h0, h1, b_out,
               sem_in, sem_out):
        copy = pltpu.make_async_copy

        def cp_awqkv(p):
            cols = pl.ds(p * D, D)
            return copy(awqkv_hbm.at[:, cols], awqkv_raw.at[:, cols], sem_in.at[sem_aw + p])

        def cp_ax(c, n, sem):
            rows = pl.ds(pl.multiple_of(c * A_CHUNK, A_CHUNK), n * A_CHUNK)
            return copy(ax_hbm.at[rows], ax.at[rows], sem_in.at[sem])

        def cps_pair(g, with_x):
            cps = [cp_ax(g + 2, 1, sem_pair + g)] if with_x else []
            return cps + [copy(w.at[g], wraw.at[j, g], sem_in.at[sem_pair + g])
                          for j, w in enumerate((wq_hbm, wk_hbm, wv_hbm))]

        def cp_wo(i):
            grp = pl.ds(pl.multiple_of(i * WO_GROUP, WO_GROUP), WO_GROUP)
            return copy(wo_hbm.at[grp], wo_raw.at[grp], sem_in.at[sem_wo + i])

        def cp_bout(i):
            rows = pl.ds(pl.multiple_of(i * B_UNROLL * seg, B_UNROLL * seg), B_UNROLL * seg)
            return copy(b_out.at[rows], out_hbm.at[rows, pl.ds(D, D)], sem_out.at[1])

        cp_ax0 = cp_ax(0, 2, sem_ax)
        cp_awo = copy(awo_hbm, awo_raw, sem_in.at[sem_awo])
        cps_b0 = [copy(mem_hbm, mem0, sem_in.at[sem_bx0]),
                  copy(bx_hbm.at[:, pl.ds(seg - B_EARLY, B_EARLY), :], bxe, sem_in.at[sem_bx0])]
        cp_bx_head, cp_bx_rest = (
            copy(bx_hbm.at[segs], bx.at[segs], sem_in.at[sem])
            for segs, sem in ((pl.ds(0, B_UNROLL), sem_bx1), (pl.ds(B_UNROLL, n_seg - B_UNROLL), sem_bx2)))
        cp_aout = copy(a_out, out_hbm.at[:, pl.ds(0, D)], sem_out.at[0])
        n_iter = n_chunk // 2 - 1

        early = [cp_awqkv(0), cp_ax0, cp_awqkv(1), cp_awqkv(2), cp_awo]
        late = []
        for g in range(n_chunk - 2):
            (early if g < n_pair // 2 else late).extend(cps_pair(g, True))
        late += cps_b0
        for i in range(n_group):
            late.append(cp_wo(i))
            if n_pair - n_group + i >= n_chunk - 2:
                late += cps_pair(n_pair - n_group + i, False)
        late += [cp_bx_head, cp_bx_rest]
        for cp in early:
            cp.start()

        def reorder(src, dst, base, j):
            for t in range(nt_d):
                x = src[t, pl.ds(base + j, A_HEADS, stride=a_dh // 2), :]
                even = pltpu.bitcast(x << 16, F32)
                odd = pltpu.bitcast((x >> 16) << 16, F32)
                y = jnp.concatenate([even, odd], axis=0).astype(BF16)
                dst[pl.ds(base + A_HEADS * j, A_HEADS), _tile(t)] = pltpu.bitcast(y, U32)

        def a_proj(c, buf, n):
            x = ax[pl.ds(pl.multiple_of(c * A_CHUNK, A_CHUNK), A_CHUNK), :]
            w = pltpu.bitcast(awp[n * (LANES // 2):(n + 1) * (LANES // 2), :], BF16)
            r = _nt(x, w)
            buf[n, A_HALO:, :] = r

        def a_halo(cur, nxt):
            for n in range(nt_d, 3 * nt_d):
                nxt[n, 0:A_HALO, :] = cur[n, A_CHUNK:A_CHUNK + A_HALO, :]

        def a_attn(c, buf, o):
            st = {}

            def dots(r):
                qs = [buf[t, A_HALO + 8 * r:A_HALO + 8 * r + 8, :] for t in range(nt_d)]
                st[r] = []
                for w in range(A_WIN):
                    off = A_HALO + 8 * r - A_DIL * w
                    s = qs[0] * buf[nt_d, off:off + 8, :]
                    for t in range(1, nt_d):
                        s = s + qs[t] * buf[nt_d + t, off:off + 8, :]
                    st[r].append(s + pltpu.roll(s, 2 * A_HEADS, 1))

            def fold(r):
                st[r] = [s + pltpu.roll(s, A_HEADS, 1) for s in st[r]]

            def mix(r):
                logits = []
                for w, s in enumerate(st.pop(r)):
                    s = s * a_scale
                    if 8 * r < A_DIL * w:
                        pos = c * A_CHUNK + 8 * r + lax.broadcasted_iota(jnp.int32, (8, LANES), 0)
                        s = jnp.where(pos >= A_DIL * w, s, NEG)
                    logits.append(s)
                m = functools.reduce(jnp.maximum, logits)
                es = [jnp.exp(s - m) for s in logits]
                inv = 1.0 / functools.reduce(jnp.add, es)
                ps = [e * inv for e in es]
                for t in range(nt_d):
                    acc = None
                    for w in range(A_WIN):
                        off = A_HALO + 8 * r - A_DIL * w
                        term = ps[w] * buf[2 * nt_d + t, off:off + 8, :]
                        acc = term if acc is None else acc + term
                    o[8 * r:8 * r + 8, _tile(t)] = acc

            return _pipeline(A_CHUNK // 8, ((fold, 1), (dots, 0), (mix, 2)))

        def a_oproj(c, o, t):
            r = _nn(o[...], pltpu.bitcast(awop[:, _tile(t)], BF16))
            a_out[pl.ds(pl.multiple_of(c * A_CHUNK, A_CHUNK), A_CHUNK), _tile(t)] = r.astype(BF16)

        def b_prep(g):
            def slab(i):
                j, t = divmod(i, PW // LANES)
                wqkv[g, :, _tile(i)] = pltpu.bitcast(wraw[j, g, _tile(t), :].T, U32)
            return [part(slab, i) for i in range(3 * PW // LANES)]

        def proj_tasks(c, bufs):
            return [part(a_proj, c, bufs, n) for n in range(3 * nt_d)]

        def oproj_tasks(c, o):
            return [part(a_oproj, c, o, t) for t in range(nt_d)]

        buf0, buf1 = qkv0, qkv1
        nxt_proj = proj_tasks(1, buf1)
        for p in range(3):
            cp_awqkv(p).wait()
            if p > 0:
                _run(nxt_proj[(p - 1) * nt_d:p * nt_d])
            for t in range(nt_d):
                aw_t[t, pl.ds(p * D // 2, D // 2), :] = pltpu.bitcast(
                    awqkv_raw[_tile(t), p * D:(p + 1) * D].T, U32)
            if p == 0:
                cp_ax0.wait()
            for t in range(nt_d):
                reorder(aw_t, awp, p * D // 2, 2 * t)
                reorder(aw_t, awp, p * D // 2, 2 * t + 1)
                a_proj(0, buf0, p * nt_d + t)
        cp_awo.wait()
        for t in range(nt_d):
            for n in (nt_d + t, 2 * nt_d + t):
                buf0[n, 0:A_HALO, :] = jnp.broadcast_to(buf0[n, A_HALO:A_HALO + 1, :], (A_HALO, LANES))
            awo_t[t, 0:D // 2, :] = pltpu.bitcast(awo_raw[:, _tile(t)], U32)
        a_halo(buf0, buf1)
        _run(_interleave(nxt_proj[2 * nt_d:], a_attn(0, buf0, o0),
                         [part(reorder, awo_t, awop, 0, j) for j in range(a_dh // 2)]))
        for cp in late:
            cp.start()

        def a_body(i, carry):
            for c, cur, nxt, o_cur, o_prev in ((2 * i + 1, buf1, buf0, o1, o0), (2 * i + 2, buf0, buf1, o0, o1)):
                for cp in cps_pair(c - 1, True):
                    cp.wait()
                a_halo(cur, nxt)
                _run(_interleave(oproj_tasks(c - 1, o_prev) + proj_tasks(c + 1, nxt),
                                 a_attn(c, cur, o_cur) + b_prep(c - 1)))
            return carry

        lax.fori_loop(0, n_iter, a_body, 0)

        def b_step(s, h_ref, h_next, chained):
            r0 = pl.multiple_of(s * seg, seg)
            h_ref[M:L, :] = bx[s].astype(F32)
            low = lax.broadcasted_iota(jnp.int32, (L, LANES), 1) < Dh - LANES
            col = lax.broadcasted_iota(jnp.int32, (L, 2 * L), 1)
            row = lax.broadcasted_iota(jnp.int32, (L, 2 * L), 0)
            first = col < L
            allow = (row < M) | (row >= jnp.where(first, col, col - L))
            zero = jnp.zeros((L, LANES), F32)

            def blockdiag(x):
                t0, t1, t2 = x[:, _tile(0)], x[:, _tile(1)], x[:, _tile(2)]
                top = jnp.concatenate([t0, jnp.where(low, t1, 0.0), zero], axis=1)
                bot = jnp.concatenate([zero, jnp.where(low, 0.0, t1), t2], axis=1)
                return jnp.concatenate([top, bot], axis=0).astype(BF16)

            st = {}

            def proj(g):
                lo = PW if g < B_EARLY_SETS * n_group else 0
                if chained and g == 0:
                    r = None
                    for t in range(nt_d):
                        w = pltpu.bitcast(wqkv[g, t * (LANES // 2):(t + 1) * (LANES // 2), lo:], BF16)
                        term = _nn(h_ref[:, _tile(t)], w)
                        r = term if r is None else r + term
                else:
                    r = _nn(h_ref[...], pltpu.bitcast(wqkv[g, :, lo:], BF16))
                if lo:
                    q = _nn(h_ref[0:L - B_EARLY, :], pltpu.bitcast(wqkv[g, :, 0:PW], BF16))
                    rows = pl.ds(pl.multiple_of(s * B_EARLY, B_EARLY), B_EARLY)
                    r = jnp.concatenate([jnp.concatenate([q, early_q[g, rows, :]], axis=0), r], axis=1)
                st[g] = dict(q=r[:, 0:PW], k=blockdiag(r[:, PW:2 * PW]), v=blockdiag(r[:, 2 * PW:3 * PW]))

            def scores(g):
                d = st[g]
                sc = jnp.where(allow, _nt(d['q'], d['k']) * b_scale, NEG)
                m0 = jnp.max(jnp.where(first, sc, -jnp.inf), axis=1, keepdims=True)
                m1 = jnp.max(jnp.where(first, -jnp.inf, sc), axis=1, keepdims=True)
                e = jnp.exp(sc - jnp.where(first, m0, m1))
                l0 = jnp.sum(jnp.where(first, e, 0.0), axis=1, keepdims=True)
                l1 = jnp.sum(jnp.where(first, 0.0, e), axis=1, keepdims=True)
                d['p'] = e / jnp.where(first, l0, l1)

            def mix(g):
                d = st[g]
                d['o'] = _nn(d['p'], d['v'])

            def oproj(g):
                if g == n_pair - 2:
                    return
                if g == n_pair - 1:
                    o = jnp.concatenate([st.pop(j)['o'] for j in range(n_pair - 2, n_pair)], axis=1)
                    w = jnp.concatenate([pltpu.bitcast(wo[j], BF16) for j in range(n_pair - 2, n_pair)], axis=0)
                    r = _nn(o, w)
                else:
                    r = _nn(st.pop(g)['o'], pltpu.bitcast(wo[g], BF16))
                st['acc'] = st['acc'] + r if g else r

            def finish():
                out = st.pop('acc')
                for t in range(nt_d):
                    h_next[0:M, _tile(t)] = out[0:M, _tile(t)].astype(BF16).astype(F32)
                b_out[pl.ds(r0, seg), :] = out[M:L].astype(BF16)

            stages = ((proj, 0), (scores, 1), (mix, 4), (oproj, 7))
            return _pipeline(n_pair, stages) + [finish]

        for cp in cps_b0:
            cp.wait()
        h0[0:M, :] = mem0[...].astype(F32)
        for s in range(0, n_seg, 2):
            x = jnp.concatenate([bxe[s].astype(F32), bxe[s + 1].astype(F32)], axis=0)
            xe[s * B_EARLY // 2:(s + 2) * B_EARLY // 2, :] = pltpu.bitcast(x.astype(BF16), U32)
        _run(_interleave(oproj_tasks(n_chunk - 2, o0), a_attn(n_chunk - 1, buf1, o1)))
        _run(oproj_tasks(n_chunk - 1, o1))

        def early_body(i, carry):
            cp_wo(i).wait()

            @pl.when(n_pair - n_group + i >= n_chunk - 2)
            def _():
                for cp in cps_pair(n_pair - n_group + i, False):
                    cp.wait()

            def project(e, n):
                early_q[e * n_group + i, :, _tile(n)] = _nn(
                    pltpu.bitcast(xe[...], BF16), pltpu.bitcast(wqkv[e * n_group + i, :, _tile(n)], BF16))

            def retile(j):
                wo[i * WO_GROUP + j] = pltpu.bitcast(wo_raw[i * WO_GROUP + j], U32)

            _run(_interleave([part(project, e, n) for e in range(B_EARLY_SETS) for n in range(PW // LANES)],
                             [part(retile, j) for j in range(WO_GROUP)],
                             b_prep(n_pair - n_group + i)))
            return carry

        lax.fori_loop(0, n_group, early_body, 0)
        cp_bx_head.wait()
        cp_aout.start()

        def b_body(i, carry):
            for u in range(B_UNROLL):
                _run(b_step(B_UNROLL * i + u, (h0, h1)[u % 2], (h1, h0)[u % 2], chained=u > 0))

            @pl.when(i == 0)
            def _():
                cp_bx_rest.wait()

            @pl.when(i > 0)
            def _():
                cp_bout(i - 1).wait()

            cp_bout(i).start()
            return carry

        lax.fori_loop(0, n_seg // B_UNROLL, b_body, 0)
        cp_aout.wait()
        cp_bout(n_seg // B_UNROLL - 1).wait()

    qkvbuf = pltpu.VMEM((3 * nt_d, A_HALO + A_CHUNK, LANES), F32)
    obuf = pltpu.VMEM((A_CHUNK, D), F32)
    hbuf = pltpu.VMEM((L, D), F32)
    scratch = [
        pltpu.VMEM((S, D), BF16),
        pltpu.VMEM((D, 3 * D), BF16),
        pltpu.VMEM((D, D), BF16),
        pltpu.VMEM((nt_d, 3 * D // 2 + 16, LANES), U32),
        pltpu.VMEM((3 * D // 2, D), U32),
        pltpu.VMEM((nt_d, D // 2 + 16, LANES), U32),
        pltpu.VMEM((D // 2, D), U32),
        qkvbuf, qkvbuf, obuf, obuf,
        pltpu.VMEM((S, D), BF16),
        pltpu.VMEM((n_seg, seg, D), BF16),
        pltpu.VMEM((n_seg, B_EARLY, D), BF16),
        pltpu.VMEM((n_seg * B_EARLY // 2, D), U32),
        pltpu.VMEM((n_group * B_EARLY_SETS, n_seg * B_EARLY, PW), F32),
        pltpu.VMEM((M, D), BF16),
        pltpu.VMEM((3, n_pair, PW, D), BF16),
        pltpu.VMEM((n_pair, PW, D), BF16),
        pltpu.VMEM((n_pair, D // 2, 3 * PW), U32),
        pltpu.VMEM((n_pair, PW // 2, D), U32),
        hbuf, hbuf,
        pltpu.VMEM((S, D), BF16),
        pltpu.SemaphoreType.DMA((sem_wo + n_group,)),
        pltpu.SemaphoreType.DMA((2,)),
    ]
    return pl.pallas_call(
        kernel,
        out_shape=jax.ShapeDtypeStruct((S, 2 * D), BF16),
        in_specs=[pl.BlockSpec(memory_space=pl.ANY)] * 9,
        out_specs=pl.BlockSpec(memory_space=pl.ANY),
        scratch_shapes=scratch,
        compiler_params=pltpu.CompilerParams(vmem_limit_bytes=110 * 1024 * 1024),
    )


@functools.partial(jax.jit, static_argnames=("B_seg_len",))
def pallas_concat_heads__sliding_local_dilated__memory_aug_recurrent_mem_tr__prompt_kernel(
    A_x, A_wqkv, A_wo, B_x, B_mem0, B_Wq, B_Wk, B_Wv, B_Wo, B_seg_len,
):
    batch, S, D = B_x.shape
    M = B_mem0.shape[1]
    _, H, Dh = B_Wq.shape
    assert batch == 1 and A_x.shape == B_x.shape

    def pairs(w):
        return jnp.transpose(w, (1, 2, 0)).reshape(H // 2, 2 * Dh, D)

    seg = int(B_seg_len)
    out = _build(S, D, M, H, Dh, seg)(
        A_x.reshape(S, D), A_wqkv, A_wo, B_x.reshape(S // seg, seg, D), B_mem0.reshape(M, D),
        pairs(B_Wq), pairs(B_Wk), pairs(B_Wv), B_Wo.reshape(H // 2, 2 * Dh, D))
    return out.reshape(1, S, 2 * D)
```

```python
import functools

import jax
import jax.numpy as jnp
from jax import lax
import jax.experimental.pallas as pl
import jax.experimental.pallas.tpu as pltpu

F32 = jnp.float32
BF16 = jnp.bfloat16
U32 = jnp.uint32

LANES = 128
A_HEADS = 32
A_WIN = 8
A_DIL = 2
A_CHUNK = 128
A_HALO = 16
B_UNROLL = 4
B_EARLY = 8
B_EARLY_SETS = 3
WO_GROUP = 4
NEG = -1000000000.0


def _nn(a, b):
    return lax.dot_general(a, b, (((1,), (0,)), ((), ())), preferred_element_type=F32)


def _nt(a, b):
    return lax.dot_general(a, b, (((1,), (1,)), ((), ())), preferred_element_type=F32)


def _tile(t):
    return slice(t * LANES, (t + 1) * LANES)


def _interleave(*lists):
    keyed = [((i + 0.5) / len(tasks), k, f) for k, tasks in enumerate(lists) for i, f in enumerate(tasks)]
    return [f for _, _, f in sorted(keyed, key=lambda e: e[:2])]


def _pipeline(n, stages):
    def slot(t):
        for fn, lag in stages:
            if 0 <= t - lag < n:
                fn(t - lag)
    return [functools.partial(slot, t) for t in range(n + max(lag for _, lag in stages))]


def _run(tasks):
    for f in tasks:
        f()


def _build(S, D, M, H, Dh, seg):
    nt_d = D // LANES
    a_dh = D // A_HEADS
    n_chunk = S // A_CHUNK
    n_pair = H // 2
    PW = 2 * Dh
    L = M + seg
    n_seg = S // seg
    assert D % LANES == 0 and 4 * A_HEADS == LANES and a_dh == 4 * nt_d
    assert PW == 3 * LANES and n_pair == n_chunk and n_chunk % 2 == 0
    assert M % 8 == 0 and seg % 16 == 0 and 2 * L <= LANES
    assert n_seg % B_UNROLL == 0 and B_UNROLL % 2 == 0 and n_pair % WO_GROUP == 0
    n_group = n_pair // WO_GROUP
    assert (B_EARLY_SETS + 1) * n_group <= n_pair
    sem_ax, sem_awo, sem_bx0, sem_bx, sem_aw = range(5)
    sem_pair = sem_aw + 3
    sem_wo = sem_pair + n_pair
    a_scale = a_dh ** -0.5
    b_scale = Dh ** -0.5
    part = functools.partial

    def kernel(ax_hbm, awqkv_hbm, awo_hbm, bx_hbm, mem_hbm, wq_hbm, wk_hbm, wv_hbm, wo_hbm,
               out_hbm,
               ax, awqkv_raw, awo_raw, aw_t, awp, awo_t, awop,
               qkv0, qkv1, o0, o1, a_out,
               bx, bxe, xe, early_q, mem0, wraw, wo_raw, wqkv, wo, h0, h1, b_out,
               sem_in, sem_out):
        copy = pltpu.make_async_copy

        def cp_awqkv(p):
            cols = pl.ds(p * D, D)
            return copy(awqkv_hbm.at[:, cols], awqkv_raw.at[:, cols], sem_in.at[sem_aw + p])

        def cp_ax(c, n, sem):
            rows = pl.ds(pl.multiple_of(c * A_CHUNK, A_CHUNK), n * A_CHUNK)
            return copy(ax_hbm.at[rows], ax.at[rows], sem_in.at[sem])

        def cps_pair(g, with_x):
            cps = [cp_ax(g + 2, 1, sem_pair + g)] if with_x else []
            return cps + [copy(w.at[g], wraw.at[j, g], sem_in.at[sem_pair + g])
                          for j, w in enumerate((wq_hbm, wk_hbm, wv_hbm))]

        def cp_wo(i):
            grp = pl.ds(pl.multiple_of(i * WO_GROUP, WO_GROUP), WO_GROUP)
            return copy(wo_hbm.at[grp], wo_raw.at[grp], sem_in.at[sem_wo + i])

        def cp_bout(i):
            rows = pl.ds(pl.multiple_of(i * B_UNROLL * seg, B_UNROLL * seg), B_UNROLL * seg)
            return copy(b_out.at[rows], out_hbm.at[rows, pl.ds(D, D)], sem_out.at[1])

        cp_ax0 = cp_ax(0, 2, sem_ax)
        cp_awo = copy(awo_hbm, awo_raw, sem_in.at[sem_awo])
        cps_b0 = [copy(mem_hbm, mem0, sem_in.at[sem_bx0]),
                  copy(bx_hbm.at[:, pl.ds(seg - B_EARLY, B_EARLY), :], bxe, sem_in.at[sem_bx0])]
        cp_bx = copy(bx_hbm, bx, sem_in.at[sem_bx])
        cp_aout = copy(a_out, out_hbm.at[:, pl.ds(0, D)], sem_out.at[0])
        n_iter = n_chunk // 2 - 1

        early = [cp_awqkv(0), cp_ax0, cp_awqkv(1), cp_awqkv(2), cp_awo]
        late = []
        for g in range(n_chunk - 2):
            (early if g < n_pair // 2 else late).extend(cps_pair(g, True))
        late += cps_b0
        for i in range(n_group):
            late.append(cp_wo(i))
            if n_pair - n_group + i >= n_chunk - 2:
                late += cps_pair(n_pair - n_group + i, False)
        late.append(cp_bx)
        for cp in early:
            cp.start()

        def reorder(src, dst, base, j):
            for t in range(nt_d):
                x = src[t, pl.ds(base + j, A_HEADS, stride=a_dh // 2), :]
                even = pltpu.bitcast(x << 16, F32)
                odd = pltpu.bitcast((x >> 16) << 16, F32)
                y = jnp.concatenate([even, odd], axis=0).astype(BF16)
                dst[pl.ds(base + A_HEADS * j, A_HEADS), _tile(t)] = pltpu.bitcast(y, U32)

        def a_proj(c, buf, n):
            x = ax[pl.ds(pl.multiple_of(c * A_CHUNK, A_CHUNK), A_CHUNK), :]
            w = pltpu.bitcast(awp[n * (LANES // 2):(n + 1) * (LANES // 2), :], BF16)
            r = _nt(x, w)
            buf[n, A_HALO:, :] = r

        def a_halo(cur, nxt):
            for n in range(nt_d, 3 * nt_d):
                nxt[n, 0:A_HALO, :] = cur[n, A_CHUNK:A_CHUNK + A_HALO, :]

        def a_attn(c, buf, o):
            st = {}

            def dots(r):
                qs = [buf[t, A_HALO + 8 * r:A_HALO + 8 * r + 8, :] for t in range(nt_d)]
                st[r] = []
                for w in range(A_WIN):
                    off = A_HALO + 8 * r - A_DIL * w
                    s = qs[0] * buf[nt_d, off:off + 8, :]
                    for t in range(1, nt_d):
                        s = s + qs[t] * buf[nt_d + t, off:off + 8, :]
                    st[r].append(s + pltpu.roll(s, 2 * A_HEADS, 1))

            def fold(r):
                st[r] = [s + pltpu.roll(s, A_HEADS, 1) for s in st[r]]

            def mix(r):
                logits = []
                for w, s in enumerate(st.pop(r)):
                    s = s * a_scale
                    if 8 * r < A_DIL * w:
                        pos = c * A_CHUNK + 8 * r + lax.broadcasted_iota(jnp.int32, (8, LANES), 0)
                        s = jnp.where(pos >= A_DIL * w, s, NEG)
                    logits.append(s)
                m = functools.reduce(jnp.maximum, logits)
                es = [jnp.exp(s - m) for s in logits]
                inv = 1.0 / functools.reduce(jnp.add, es)
                ps = [e * inv for e in es]
                for t in range(nt_d):
                    acc = None
                    for w in range(A_WIN):
                        off = A_HALO + 8 * r - A_DIL * w
                        term = ps[w] * buf[2 * nt_d + t, off:off + 8, :]
                        acc = term if acc is None else acc + term
                    o[8 * r:8 * r + 8, _tile(t)] = acc

            return _pipeline(A_CHUNK // 8, ((fold, 1), (dots, 0), (mix, 2)))

        def a_oproj(c, o, t):
            r = _nn(o[...], pltpu.bitcast(awop[:, _tile(t)], BF16))
            a_out[pl.ds(pl.multiple_of(c * A_CHUNK, A_CHUNK), A_CHUNK), _tile(t)] = r.astype(BF16)

        def b_prep(g):
            def slab(i):
                j, t = divmod(i, PW // LANES)
                wqkv[g, :, _tile(i)] = pltpu.bitcast(wraw[j, g, _tile(t), :].T, U32)
            return [part(slab, i) for i in range(3 * PW // LANES)]

        def proj_tasks(c, bufs):
            return [part(a_proj, c, bufs, n) for n in range(3 * nt_d)]

        def oproj_tasks(c, o):
            return [part(a_oproj, c, o, t) for t in range(nt_d)]

        buf0, buf1 = qkv0, qkv1
        nxt_proj = proj_tasks(1, buf1)
        for p in range(3):
            cp_awqkv(p).wait()
            if p > 0:
                _run(nxt_proj[(p - 1) * nt_d:p * nt_d])
            for t in range(nt_d):
                aw_t[t, pl.ds(p * D // 2, D // 2), :] = pltpu.bitcast(
                    awqkv_raw[_tile(t), p * D:(p + 1) * D].T, U32)
            if p == 0:
                cp_ax0.wait()
            for t in range(nt_d):
                reorder(aw_t, awp, p * D // 2, 2 * t)
                reorder(aw_t, awp, p * D // 2, 2 * t + 1)
                a_proj(0, buf0, p * nt_d + t)
        cp_awo.wait()
        for t in range(nt_d):
            for n in (nt_d + t, 2 * nt_d + t):
                buf0[n, 0:A_HALO, :] = jnp.broadcast_to(buf0[n, A_HALO:A_HALO + 1, :], (A_HALO, LANES))
            awo_t[t, 0:D // 2, :] = pltpu.bitcast(awo_raw[:, _tile(t)], U32)
        a_halo(buf0, buf1)
        _run(_interleave(nxt_proj[2 * nt_d:], a_attn(0, buf0, o0),
                         [part(reorder, awo_t, awop, 0, j) for j in range(a_dh // 2)]))
        for cp in late:
            cp.start()

        def a_body(i, carry):
            for c, cur, nxt, o_cur, o_prev in ((2 * i + 1, buf1, buf0, o1, o0), (2 * i + 2, buf0, buf1, o0, o1)):
                for cp in cps_pair(c - 1, True):
                    cp.wait()
                a_halo(cur, nxt)
                _run(_interleave(oproj_tasks(c - 1, o_prev) + proj_tasks(c + 1, nxt),
                                 a_attn(c, cur, o_cur) + b_prep(c - 1)))
            return carry

        lax.fori_loop(0, n_iter, a_body, 0)

        def b_step(s, h_ref, h_next, chained):
            r0 = pl.multiple_of(s * seg, seg)
            h_ref[M:L, :] = bx[s].astype(F32)
            low = lax.broadcasted_iota(jnp.int32, (L, LANES), 1) < Dh - LANES
            col = lax.broadcasted_iota(jnp.int32, (L, 2 * L), 1)
            row = lax.broadcasted_iota(jnp.int32, (L, 2 * L), 0)
            first = col < L
            allow = (row < M) | (row >= jnp.where(first, col, col - L))
            zero = jnp.zeros((L, LANES), F32)

            def blockdiag(x):
                t0, t1, t2 = x[:, _tile(0)], x[:, _tile(1)], x[:, _tile(2)]
                top = jnp.concatenate([t0, jnp.where(low, t1, 0.0), zero], axis=1)
                bot = jnp.concatenate([zero, jnp.where(low, 0.0, t1), t2], axis=1)
                return jnp.concatenate([top, bot], axis=0).astype(BF16)

            st = {}

            def proj(g):
                lo = PW if g < B_EARLY_SETS * n_group else 0
                if chained and g == 0:
                    r = None
                    for t in range(nt_d):
                        w = pltpu.bitcast(wqkv[g, t * (LANES // 2):(t + 1) * (LANES // 2), lo:], BF16)
                        term = _nn(h_ref[:, _tile(t)], w)
                        r = term if r is None else r + term
                else:
                    r = _nn(h_ref[...], pltpu.bitcast(wqkv[g, :, lo:], BF16))
                if lo:
                    q = _nn(h_ref[0:L - B_EARLY, :], pltpu.bitcast(wqkv[g, :, 0:PW], BF16))
                    rows = pl.ds(pl.multiple_of(s * B_EARLY, B_EARLY), B_EARLY)
                    r = jnp.concatenate([jnp.concatenate([q, early_q[g, rows, :]], axis=0), r], axis=1)
                st[g] = dict(q=r[:, 0:PW], k=blockdiag(r[:, PW:2 * PW]), v=blockdiag(r[:, 2 * PW:3 * PW]))

            def scores(g):
                d = st[g]
                sc = jnp.where(allow, _nt(d['q'], d['k']) * b_scale, NEG)
                m0 = jnp.max(jnp.where(first, sc, -jnp.inf), axis=1, keepdims=True)
                m1 = jnp.max(jnp.where(first, -jnp.inf, sc), axis=1, keepdims=True)
                e = jnp.exp(sc - jnp.where(first, m0, m1))
                l0 = jnp.sum(jnp.where(first, e, 0.0), axis=1, keepdims=True)
                l1 = jnp.sum(jnp.where(first, 0.0, e), axis=1, keepdims=True)
                d['p'] = e / jnp.where(first, l0, l1)

            def mix(g):
                d = st[g]
                d['o'] = _nn(d['p'], d['v'])

            def oproj(g):
                if g == n_pair - 2:
                    return
                if g == n_pair - 1:
                    o = jnp.concatenate([st.pop(j)['o'] for j in range(n_pair - 2, n_pair)], axis=1)
                    w = jnp.concatenate([pltpu.bitcast(wo[j], BF16) for j in range(n_pair - 2, n_pair)], axis=0)
                    r = _nn(o, w)
                else:
                    r = _nn(st.pop(g)['o'], pltpu.bitcast(wo[g], BF16))
                st['acc'] = st['acc'] + r if g else r

            def finish():
                out = st.pop('acc')
                for t in range(nt_d):
                    h_next[0:M, _tile(t)] = out[0:M, _tile(t)].astype(BF16).astype(F32)
                b_out[pl.ds(r0, seg), :] = out[M:L].astype(BF16)

            stages = ((proj, 0), (scores, 1), (mix, 4), (oproj, 7))
            return _pipeline(n_pair, stages) + [finish]

        for cp in cps_b0:
            cp.wait()
        h0[0:M, :] = mem0[...].astype(F32)
        for s in range(0, n_seg, 2):
            x = jnp.concatenate([bxe[s].astype(F32), bxe[s + 1].astype(F32)], axis=0)
            xe[s * B_EARLY // 2:(s + 2) * B_EARLY // 2, :] = pltpu.bitcast(x.astype(BF16), U32)
        _run(_interleave(oproj_tasks(n_chunk - 2, o0), a_attn(n_chunk - 1, buf1, o1)))
        _run(oproj_tasks(n_chunk - 1, o1))

        def early_body(i, carry):
            cp_wo(i).wait()

            @pl.when(n_pair - n_group + i >= n_chunk - 2)
            def _():
                for cp in cps_pair(n_pair - n_group + i, False):
                    cp.wait()

            def project(e, n):
                early_q[e * n_group + i, :, _tile(n)] = _nn(
                    pltpu.bitcast(xe[...], BF16), pltpu.bitcast(wqkv[e * n_group + i, :, _tile(n)], BF16))

            def retile(j):
                wo[i * WO_GROUP + j] = pltpu.bitcast(wo_raw[i * WO_GROUP + j], U32)

            _run(_interleave([part(project, e, n) for e in range(B_EARLY_SETS) for n in range(PW // LANES)],
                             [part(retile, j) for j in range(WO_GROUP)],
                             b_prep(n_pair - n_group + i)))
            return carry

        lax.fori_loop(0, n_group, early_body, 0)
        cp_bx.wait()
        cp_aout.start()

        def b_body(i, carry):
            for u in range(B_UNROLL):
                _run(b_step(B_UNROLL * i + u, (h0, h1)[u % 2], (h1, h0)[u % 2], chained=u > 0))

            @pl.when(i > 0)
            def _():
                cp_bout(i - 1).wait()

            cp_bout(i).start()
            return carry

        lax.fori_loop(0, n_seg // B_UNROLL, b_body, 0)
        cp_aout.wait()
        cp_bout(n_seg // B_UNROLL - 1).wait()

    qkvbuf = pltpu.VMEM((3 * nt_d, A_HALO + A_CHUNK, LANES), F32)
    obuf = pltpu.VMEM((A_CHUNK, D), F32)
    hbuf = pltpu.VMEM((L, D), F32)
    scratch = [
        pltpu.VMEM((S, D), BF16),
        pltpu.VMEM((D, 3 * D), BF16),
        pltpu.VMEM((D, D), BF16),
        pltpu.VMEM((nt_d, 3 * D // 2 + 16, LANES), U32),
        pltpu.VMEM((3 * D // 2, D), U32),
        pltpu.VMEM((nt_d, D // 2 + 16, LANES), U32),
        pltpu.VMEM((D // 2, D), U32),
        qkvbuf, qkvbuf, obuf, obuf,
        pltpu.VMEM((S, D), BF16),
        pltpu.VMEM((n_seg, seg, D), BF16),
        pltpu.VMEM((n_seg, B_EARLY, D), BF16),
        pltpu.VMEM((n_seg * B_EARLY // 2, D), U32),
        pltpu.VMEM((n_group * B_EARLY_SETS, n_seg * B_EARLY, PW), F32),
        pltpu.VMEM((M, D), BF16),
        pltpu.VMEM((3, n_pair, PW, D), BF16),
        pltpu.VMEM((n_pair, PW, D), BF16),
        pltpu.VMEM((n_pair, D // 2, 3 * PW), U32),
        pltpu.VMEM((n_pair, PW // 2, D), U32),
        hbuf, hbuf,
        pltpu.VMEM((S, D), BF16),
        pltpu.SemaphoreType.DMA((sem_wo + n_group,)),
        pltpu.SemaphoreType.DMA((2,)),
    ]
    return pl.pallas_call(
        kernel,
        out_shape=jax.ShapeDtypeStruct((S, 2 * D), BF16),
        in_specs=[pl.BlockSpec(memory_space=pl.ANY)] * 9,
        out_specs=pl.BlockSpec(memory_space=pl.ANY),
        scratch_shapes=scratch,
        compiler_params=pltpu.CompilerParams(vmem_limit_bytes=110 * 1024 * 1024),
    )


@functools.partial(jax.jit, static_argnames=("B_seg_len",))
def pallas_concat_heads__sliding_local_dilated__memory_aug_recurrent_mem_tr__prompt_kernel(
    A_x, A_wqkv, A_wo, B_x, B_mem0, B_Wq, B_Wk, B_Wv, B_Wo, B_seg_len,
):
    batch, S, D = B_x.shape
    M = B_mem0.shape[1]
    _, H, Dh = B_Wq.shape
    assert batch == 1 and A_x.shape == B_x.shape

    def pairs(w):
        return jnp.transpose(w, (1, 2, 0)).reshape(H // 2, 2 * Dh, D)

    seg = int(B_seg_len)
    out = _build(S, D, M, H, Dh, seg)(
        A_x.reshape(S, D), A_wqkv, A_wo, B_x.reshape(S // seg, seg, D), B_mem0.reshape(M, D),
        pairs(B_Wq), pairs(B_Wk), pairs(B_Wv), B_Wo.reshape(H // 2, 2 * Dh, D))
    return out.reshape(1, S, 2 * D)
```
